```python
import os as _os
_os.environ.setdefault('JAX_PLATFORMS', 'cpu')
import jax
import jax.numpy as jnp

def _softmax(x, axis=-1):
    return jax.nn.softmax(x, axis=axis)

def _gelu(x):
    return jax.nn.gelu(x, approximate=True)

def _silu(x):
    return jax.nn.silu(x)

def _sigmoid(x):
    return jax.nn.sigmoid(x)

def _layernorm(x, axis=-1, eps=1e-05):
    m = jnp.mean(x, axis=axis, keepdims=True)
    v = jnp.var(x, axis=axis, keepdims=True)
    return (x - m) / jnp.sqrt(v + eps)

def _scatter_add(tgt, idx, src, axis=0):
    return tgt.at[idx].add(src)

def _segment_sum(src, seg, n):
    return jax.ops.segment_sum(src, seg, n)

class _Rng:

    def __init__(self, key):
        self._k = key

    def _next(self):
        self._k, sub = jax.random.split(self._k)
        return sub

    def normal(self, shape):
        return jax.random.normal(self._next(), shape, dtype=jnp.bfloat16)

    def randint(self, lo, hi, shape):
        return jax.random.randint(self._next(), shape, lo, hi, dtype=jnp.int32)

    def uniform(self, shape, lo=0.0, hi=1.0):
        return jax.random.uniform(self._next(), shape, jnp.bfloat16, lo, hi)

    def permutation(self, n):
        return jax.random.permutation(self._next(), n)
kernel_name = 'recurrent_scan__memory_aug_recurrent_mem_tr__mixer_gmlp__prompt'

def setup_inputs():
    _rng = _Rng(jax.random.key(int.from_bytes(__import__("os").urandom(4), "little")))
    _w = lambda a: (lambda t: t.astype(jnp.bfloat16) if jnp.issubdtype(t.dtype, jnp.floating) else t)(jnp.asarray(a))

    def _A_setup():
        B, S, Dm = (1, 2048, 640)
        H, Dh = (32, 128)
        M, seg = (8, 32)
        seg = min(seg, S)
        S = S // seg * seg
        return {'x': _w((lambda *s: _rng.normal(s) * 0.05)(B, S, Dm)), 'mem0': _w((lambda *s: _rng.normal(s) * 0.1)(B, M, Dm)), 'Wq': _w((lambda *s: _rng.normal(s) * 1.6)(Dm, H, Dh) * Dm ** (-0.5)), 'Wk': _w((lambda *s: _rng.normal(s) * 1.6)(Dm, H, Dh) * Dm ** (-0.5)), 'Wv': _w((lambda *s: _rng.normal(s) * 0.1)(Dm, H, Dh) * Dm ** (-0.5)), 'Wo': _w((lambda *s: _rng.normal(s) * 0.1)(H, Dh, Dm) * (H * Dh) ** (-0.5)), 'seg_len': seg}
    _A_in = _A_setup()

    def _B_setup():
        B, S, D, F = (1, 2048, 640, 1728)
        Fh = F // 2
        return {'x': _w((lambda *s: _rng.normal(s) * 0.05)(B, S, D)), 'w_in': _w((lambda *s: _rng.normal(s) * 0.8)(D, 2 * Fh)), 'w_sp': _w(0.01 * (lambda *s: _rng.normal(s) * 0.8)(S, S)), 'b_sp': _w(1.0 + 0.01 * (lambda *s: _rng.normal(s) * 0.05)(S)), 'w_out': _w((lambda *s: _rng.normal(s) * 0.05)(Fh, D))}
    _B_in = _B_setup()
    return {'A_x': _A_in['x'], 'A_mem0': _A_in['mem0'], 'A_Wq': _A_in['Wq'], 'A_Wk': _A_in['Wk'], 'A_Wv': _A_in['Wv'], 'A_Wo': _A_in['Wo'], 'A_seg_len': _A_in['seg_len'], 'B_x': _B_in['x'], 'B_w_in': _B_in['w_in'], 'B_w_sp': _B_in['w_sp'], 'B_b_sp': _B_in['b_sp'], 'B_w_out': _B_in['w_out']}

def reference(A_x, A_mem0, A_Wq, A_Wk, A_Wv, A_Wo, A_seg_len, B_x, B_w_in, B_w_sp, B_b_sp, B_w_out):

    def _A_ref(x, mem0, Wq, Wk, Wv, Wo, seg_len):
        B, S, Dm = x.shape
        H, Dh = (Wq.shape[1], Wq.shape[2])
        M = mem0.shape[1]
        scale = Dh ** (-0.5)
        n_seg = S // seg_len
        L = M + seg_len
        idx = jnp.arange(L)
        mask = (idx[:, None] < M) | (idx[:, None] >= idx[None, :])
        mem = mem0
        outs = []
        for s in range(n_seg):
            xs = x[:, s * seg_len:(s + 1) * seg_len, :].copy()
            h = jnp.concatenate([mem, xs], axis=1)
            q = jnp.einsum('btd,dhe->bhte', h, Wq)
            k = jnp.einsum('btd,dhe->bhte', h, Wk)
            v = jnp.einsum('btd,dhe->bhte', h, Wv)
            scores = jnp.einsum('bhqe,bhke->bhqk', q, k) * scale
            scores = jnp.where(mask[None, None], scores, -1000000000.0)
            p = _softmax(scores, axis=-1)
            o = jnp.einsum('bhqk,bhke->bhqe', p, v)
            o = jnp.einsum('bhte,hed->btd', o, Wo)
            mem = o[:, :M, :].copy()
            outs.append(o[:, M:, :])
        return jnp.concatenate(outs, axis=1)

    def _B_ref(x, w_in, w_sp, b_sp, w_out):
        B, S, D = x.shape
        F = w_in.shape[-1]
        Fh = F // 2
        z = _gelu(jnp.einsum('bsd,df->bsf', x, w_in))
        z1 = z[..., :Fh].copy()
        z2 = _layernorm(z[..., Fh:], axis=-1)
        g = jnp.einsum('ts,bsf->btf', w_sp, z2) + b_sp[None, :, None]
        return jnp.einsum('bsf,fd->bsd', z1 * g, w_out)
    x = A_x
    xn = _layernorm(x, axis=-1)
    s = _A_ref(xn, A_mem0, A_Wq, A_Wk, A_Wv, A_Wo, A_seg_len)
    g = _silu(_B_ref(xn, B_w_in, B_w_sp, B_b_sp, B_w_out))
    return x + s * g
```

```python
import functools
import math

import jax
import jax.numpy as jnp
from jax import lax
import jax.experimental.pallas as pl
import jax.experimental.pallas.tpu as pltpu

F32, BF16, U32 = jnp.float32, jnp.bfloat16, jnp.uint32
NT = (((1,), (1,)), ((), ()))
EPS = 1e-5
LOG2E = math.log2(math.e)

DEFAULT_FILL = {
    (0, 32): [("g", 0, 96)], (0, 33): [("g", 96, 192)], (0, 34): [("g", 192, 288)], (0, 35): [("g", 288, 352)],
    (1, 32): [("g", 352, 448)], (1, 33): [("g", 448, 544)], (1, 34): [("g", 544, 640)], (1, 35): [("g", 640, 704)],
    (2, 32): [("g", 704, 784)], (2, 33): [("g", 784, 864)], (2, 34): [], (2, 35): [("o", 0, 224)],
    (3, 32): [("o", 224, 336)], (3, 33): [("o", 336, 448)], (3, 34): [("o", 448, 544)], (3, 35): [("o", 544, 640)],
}
DEFAULT_CFG = dict(lags=(1, 3, 4), fill=DEFAULT_FILL, c1=96, c2=96, rcp_approx=True, post_norm=True)


def _gelu(x):
    c = math.sqrt(2.0 / math.pi)
    t = jnp.tanh(x * (x * x * (0.044715 * c) + c))
    hx = 0.5 * x
    return hx + hx * t


def _make_kernel(S, D, H, E, M, SEG, FH, cfg):
    L = M + SEG
    TB = 128
    NB = S // TB
    SPB = TB // SEG
    XB = 512
    NXB = S // XB
    KH = S // 2
    HP = H // 2
    lag_s, lag_p, lag_o = cfg["lags"]
    fill = cfg["fill"]
    C1, C2 = cfg["c1"], cfg["c2"]
    NWC = 4

    def kernel(x_hbm, mem_hbm, wq_hbm, wk_hbm, wv_hbm, wo_hbm, win_hbm, wsp_hbm, bsp_hbm, wout_hbm,
               o_hbm,
               x_v, xn_u, win_v, raw_u, wqkv_u, wo_u, wspa_v, wspb_v, z1_v, z2_u, z2raw_v, gpre_v,
               wout_v, woutt_u, mem_v, bsp_v, bsp_f, y_u, gate_v, s_v, out_v,
               sem_x, sem_win, sem_small, sem_grp, sem_wo, sem_spb, sem_out):

        def cp_x(i):
            r = pl.ds(i * XB, XB)
            return pltpu.make_async_copy(x_hbm.at[r], x_v.at[r], sem_x.at[i])

        def cp_win(c):
            n = 2 * FH // NWC
            r = pl.ds(((c + NWC // 2) % NWC) * n, n)
            return pltpu.make_async_copy(win_hbm.at[r], win_v.at[r], sem_win.at[c])

        cp_mem = pltpu.make_async_copy(mem_hbm, mem_v, sem_small.at[0])
        cp_bsp = pltpu.make_async_copy(bsp_hbm, bsp_v, sem_small.at[1])
        cp_wout = pltpu.make_async_copy(wout_hbm, wout_v, sem_small.at[2])

        def cp_group(g):
            cps = []
            for m, w in enumerate((wq_hbm, wk_hbm, wv_hbm)):
                wu = w.bitcast(U32)
                for p in range(HP // NXB):
                    cps.append(pltpu.make_async_copy(
                        wu.at[:, g * (HP // NXB) + p, :], raw_u.at[g, m, p], sem_grp.at[g]))
            r = pl.ds(g * XB, XB)
            cps.append(pltpu.make_async_copy(wsp_hbm.at[r, pl.ds(0, KH)], wspa_v.at[r], sem_grp.at[g]))
            return cps

        def cp_wo(c):
            return pltpu.make_async_copy(wo_hbm.bitcast(U32).at[:, pl.ds(c * 128, 128)], wo_u.at[c], sem_wo.at[0])

        def cp_spb(g):
            r = pl.ds(g * XB, XB)
            return pltpu.make_async_copy(wsp_hbm.at[r, pl.ds(KH, KH)], wspb_v.at[r], sem_spb.at[g])

        def cp_out(j):
            r = pl.ds(pl.multiple_of(j * TB, TB), TB)
            return pltpu.make_async_copy(out_v.at[r], o_hbm.at[r], sem_out.at[0])

        cp_x(0).start()
        for c in range(NWC):
            cp_win(c).start()
        for i in range(1, NXB):
            cp_x(i).start()
        cp_mem.start()
        cp_bsp.start()
        for g in range(NXB):
            for c in cp_group(g):
                c.start()
        cp_wout.start()
        cp_spb(0).start()
        for c in range(D // 128):
            cp_wo(c).start()
        for g in range(1, NXB):
            cp_spb(g).start()

        def ln_rows(r0, n):
            x = x_v[pl.ds(r0, n), :].astype(F32)
            mu = jnp.sum(x, axis=-1, keepdims=True) * (1.0 / D)
            d = x - mu
            var = jnp.sum(d * d, axis=-1, keepdims=True) * (1.0 / D)
            xn = (d * lax.rsqrt(var + EPS)).astype(BF16)
            r2 = r0 // 2 if isinstance(r0, int) else pl.multiple_of(r0 // 2, 8)
            xn_u[pl.ds(r2, n // 2), :] = pltpu.bitcast(xn, U32)

        cp_x(0).wait()
        for r in range(0, XB, 32):
            ln_rows(r, 32)
        for c in range(NWC):
            cp_win(c).wait()

        def win_block(i, carry):
            nxt = jnp.minimum(i + 1, NXB - 1)

            @pl.when(i + 1 < NXB)
            def _():
                cp_x_dyn = pltpu.make_async_copy(
                    x_hbm.at[pl.ds(pl.multiple_of(nxt * XB, XB), XB)],
                    x_v.at[pl.ds(pl.multiple_of(nxt * XB, XB), XB)], sem_x.at[nxt])
                cp_x_dyn.wait()

            xb = pltpu.bitcast(xn_u[pl.ds(pl.multiple_of(i * (XB // 2), XB // 2), XB // 2), :], BF16)

            def zt(r0):
                return _gelu(lax.dot_general(win_v[r0:r0 + C1, :], xb, NT, preferred_element_type=F32))

            nch = FH // C1
            ssum = jnp.zeros((8, XB), F32)
            for c in range(nch):
                z = zt(FH + c * C1)
                z2raw_v[c * C1:(c + 1) * C1, :] = z
                for r in range(0, C1, 8):
                    ssum = ssum + z[r:r + 8]
            mu = jnp.sum(ssum, axis=0, keepdims=True) * (1.0 / FH)
            mu8 = jnp.broadcast_to(mu, (8, XB))
            work = []

            def var_pass(c0, c1, acc):
                for r in range(c0, c1, 8):
                    d = z2raw_v[r:r + 8, :] - mu8
                    acc = acc + d * d
                return acc

            def norm_pass(r0, r1, rs):
                for r in range(r0, r1, 16):
                    d = (z2raw_v[r:r + 16, :] - mu) * rs
                    z2_u[i, r // 2:r // 2 + 8, :] = pltpu.bitcast(d.astype(BF16), U32)

            vsum = jnp.zeros((8, XB), F32)
            rs = None
            n_ln = XB // 32
            ln_done = 0
            third = FH // 3
            for c in range(nch):
                z = zt(c * C1)
                for t in range(XB // TB):
                    z1_v[i * (XB // TB) + t, c * C1:(c + 1) * C1, :] = z[:, t * TB:(t + 1) * TB]
                ph = c * 6 // nch
                ph_next = (c + 1) * 6 // nch
                for p in range(ph, ph_next):
                    if p < 3:
                        vsum = var_pass(p * third, (p + 1) * third, vsum)
                        if p == 2:
                            var = jnp.sum(vsum, axis=0, keepdims=True) * (1.0 / FH)
                            rs = lax.rsqrt(var + EPS)
                    else:
                        norm_pass((p - 3) * third, (p - 2) * third, rs)
                while ln_done < (c + 1) * n_ln // nch:
                    ln_rows(pl.multiple_of(nxt * XB + ln_done * 32, 32), 32)
                    ln_done += 1
            return carry

        lax.fori_loop(0, NXB, win_block, 0)

        cp_mem.wait()
        cp_bsp.wait()

        def pre_block(g, carry):
            for m in range(3):
                for p in range(HP // NXB):
                    pltpu.make_async_copy(raw_u.at[g, m, p], raw_u.at[g, m, p], sem_grp.at[g]).wait()
            rg = pl.ds(pl.multiple_of(g * XB, XB), XB)
            pltpu.make_async_copy(wspa_v.at[rg], wspa_v.at[rg], sem_grp.at[g]).wait()

            units = [(m, p, r) for m in range(3) for p in range(HP // NXB) for r in range(0, D, 16)]
            nch = FH // C2
            total = nch * (XB // TB)
            done = 0
            for t in range(XB // TB):
                j = g * (XB // TB) + t
                rows = pl.ds(pl.multiple_of(j * TB, TB), TB)
                bias = bsp_f[pl.ds(j, 1), :]
                for c in range(nch):
                    acc = bias
                    for kb in range(KH // XB):
                        lhs = pltpu.bitcast(z2_u[kb, c * C2 // 2:(c + 1) * C2 // 2, :], BF16)
                        acc = acc + lax.dot_general(lhs, wspa_v[rows, kb * XB:(kb + 1) * XB], NT,
                                                    preferred_element_type=F32)
                    gpre_v[j, c * C2:(c + 1) * C2, :] = acc
                    upto = (t * nch + c + 1) * len(units) // total
                    for m, p, r in units[done:upto]:
                        xe = raw_u[g, m, p, pl.ds(r, 8, stride=2), :]
                        xo = raw_u[g, m, p, pl.ds(r + 1, 8, stride=2), :]
                        h0 = m * H + (g * (HP // NXB) + p) * 2
                        wqkv_u[h0, r // 2:r // 2 + 8, :] = (xe & 0xFFFF) | (xo << 16)
                        wqkv_u[h0 + 1, r // 2:r // 2 + 8, :] = (xe >> 16) | (xo & jnp.uint32(0xFFFF0000))
                    done = upto
            return carry

        bsp_f[...] = bsp_v[...].astype(F32)
        lax.fori_loop(0, NXB, pre_block, 0)

        cp_wout.wait()
        for kb in range(0, FH, 128):
            n = min(128, FH - kb)
            for cb in range(D // 128):
                t = wout_v[kb:kb + n, cb * 128:(cb + 1) * 128].astype(F32)
                if n < 128:
                    t = jnp.concatenate([t, jnp.zeros((128 - n, 128), F32)], axis=0)
                woutt_u[cb * 64:(cb + 1) * 64, kb:kb + 128] = pltpu.bitcast(t.T.astype(BF16), U32)
        FP = woutt_u.shape[1]
        if FP > FH:
            y_u[FH // 2:FP // 2, :] = jnp.zeros(((FP - FH) // 2, TB), U32)
        s_v[...] = jnp.zeros(s_v.shape, F32)
        gate_v[...] = jnp.zeros(gate_v.shape, F32)
        for c in range(D // 128):
            cp_wo(c).wait()

        def combine(j):
            rows = pl.ds(pl.multiple_of(j * TB, TB), TB)
            for cb in range(D // 128):
                cols = slice(cb * 128, (cb + 1) * 128)
                g = gate_v[cols, :].T
                out_v[rows, cols] = (x_v[rows, cols].astype(F32) + s_v[:, cols] * g).astype(BF16)

        def main_block(j, mem):
            @pl.when(j % (XB // TB) == 0)
            def _():
                gq = j // (XB // TB)
                rg = pl.ds(pl.multiple_of(gq * XB, XB), XB)
                pltpu.make_async_copy(wspb_v.at[rg], wspb_v.at[rg], sem_spb.at[gq]).wait()

            combine(jnp.maximum(j - 1, 0))
            rows = pl.ds(pl.multiple_of(j * TB, TB), TB)

            def filler(kind, r0, r1):
                if kind == "g":
                    acc = gpre_v[j, r0:r1, :]
                    for kb in range(KH // XB):
                        lhs = pltpu.bitcast(z2_u[KH // XB + kb, r0 // 2:r1 // 2, :], BF16)
                        acc = acc + lax.dot_general(lhs, wspb_v[rows, kb * XB:(kb + 1) * XB], NT,
                                                    preferred_element_type=F32)
                    y = (z1_v[j, r0:r1, :] * acc).astype(BF16)
                    y_u[r0 // 2:r1 // 2, :] = pltpu.bitcast(y, U32)
                else:
                    lhs = pltpu.bitcast(woutt_u[r0 // 2:r1 // 2, :], BF16)
                    o = jnp.dot(lhs, pltpu.bitcast(y_u[...], BF16), preferred_element_type=F32)
                    gate_v[r0:r1, :] = o * jax.nn.sigmoid(o)

            row = lax.broadcasted_iota(jnp.int32, (L, L), 0)
            col = lax.broadcasted_iota(jnp.int32, (L, L), 1)
            mask = (row < M) | (row >= col)

            for u in range(SPB):
                r2 = pl.multiple_of(j * (TB // 2) + u * (SEG // 2), SEG // 2)
                xs = pltpu.bitcast(xn_u[pl.ds(r2, SEG // 2), :], BF16).astype(F32)
                h = jnp.concatenate([mem, xs], axis=0)
                q, k, v, sc, o = {}, {}, {}, {}, {}
                acc = None
                for t in range(H + lag_o):
                    if t < H:
                        q[t] = jnp.dot(h, pltpu.bitcast(wqkv_u[t], BF16), preferred_element_type=F32)
                        k[t] = jnp.dot(h, pltpu.bitcast(wqkv_u[H + t], BF16), preferred_element_type=F32)
                        v[t] = jnp.dot(h, pltpu.bitcast(wqkv_u[2 * H + t], BF16), preferred_element_type=F32)
                    a = t - lag_s
                    if 0 <= a < H:
                        sc[a] = lax.dot_general(q.pop(a), k.pop(a).astype(BF16), NT, preferred_element_type=F32)
                    a = t - lag_p
                    if 0 <= a < H:
                        s = jnp.where(mask, sc.pop(a) * (E ** -0.5 * LOG2E), -1e9 * LOG2E)
                        e = jnp.exp2(s - jnp.max(s, axis=-1, keepdims=True))
                        r = pltpu.reciprocal(jnp.sum(e, axis=-1, keepdims=True), approx=cfg["rcp_approx"])
                        if cfg["post_norm"]:
                            o[a] = jnp.dot(e, v.pop(a).astype(BF16), preferred_element_type=F32) * r
                        else:
                            o[a] = jnp.dot(e * r, v.pop(a).astype(BF16), preferred_element_type=F32)
                    a = t - lag_o
                    if 0 <= a < H:
                        oo = o.pop(a)
                        r = [jnp.dot(oo, pltpu.bitcast(wo_u[c, a * (E // 2):(a + 1) * (E // 2), :], BF16),
                                     preferred_element_type=F32) for c in range(D // 128)]
                        acc = r if acc is None else [p + n for p, n in zip(acc, r)]
                    for piece in fill.get((u, t), ()):
                        filler(*piece)
                mem = jnp.concatenate([p[0:M] for p in acc], axis=1)
                for c in range(D // 128):
                    s_v[u * SEG:(u + 1) * SEG, c * 128:(c + 1) * 128] = acc[c][M:L]

            @pl.when(j > 0)
            def _():
                cp_out(j - 1).start()

            return mem

        lax.fori_loop(0, NB, main_block, mem_v[...].astype(F32))
        combine(NB - 1)
        cp_out(NB - 1).start()
        pltpu.make_async_copy(out_v, out_v, sem_out.at[0]).wait()

    FP = -(-FH // 128) * 128
    scratch = [
        pltpu.VMEM((S, D), BF16),
        pltpu.VMEM((S // 2, D), U32),
        pltpu.VMEM((2 * FH, D), BF16),
        pltpu.VMEM((NXB, 3, HP // NXB, D, E), U32),
        pltpu.VMEM((3 * H, D // 2, E), U32),
        pltpu.VMEM((D // 128, H * E // 2, 128), U32),
        pltpu.VMEM((S, KH), BF16),
        pltpu.VMEM((S, KH), BF16),
        pltpu.VMEM((NB, FH, TB), F32),
        pltpu.VMEM((NXB, FH // 2, XB), U32),
        pltpu.VMEM((FH, XB), F32),
        pltpu.VMEM((NB, FH, TB), F32),
        pltpu.VMEM((FH, D), BF16),
        pltpu.VMEM((D // 2, FP), U32),
        pltpu.VMEM((M, D), BF16),
        pltpu.VMEM((NB, TB), BF16),
        pltpu.VMEM((NB, TB), F32),
        pltpu.VMEM((FP // 2, TB), U32),
        pltpu.VMEM((D, TB), F32),
        pltpu.VMEM((TB, D), F32),
        pltpu.VMEM((S, D), BF16),
        pltpu.SemaphoreType.DMA((NXB,)),
        pltpu.SemaphoreType.DMA((NWC,)),
        pltpu.SemaphoreType.DMA((3,)),
        pltpu.SemaphoreType.DMA((NXB,)),
        pltpu.SemaphoreType.DMA((1,)),
        pltpu.SemaphoreType.DMA((NXB,)),
        pltpu.SemaphoreType.DMA((1,)),
    ]
    return kernel, scratch


def build(cfg=None, name="rmt_gmlp"):
    cfg = {**DEFAULT_CFG, **(cfg or {})}

    def fn(A_x, A_mem0, A_Wq, A_Wk, A_Wv, A_Wo, A_seg_len, B_x, B_w_in, B_w_sp, B_b_sp, B_w_out):
        B, S, D = A_x.shape
        _, H, E = A_Wq.shape
        M = A_mem0.shape[1]
        FH = B_w_out.shape[0]
        kernel, scratch = _make_kernel(S, D, H, E, M, int(A_seg_len), FH, cfg)
        hbm = pl.BlockSpec(memory_space=pltpu.HBM)
        out = pl.pallas_call(
            kernel,
            out_shape=jax.ShapeDtypeStruct((S, D), A_x.dtype),
            in_specs=[hbm] * 10,
            out_specs=hbm,
            scratch_shapes=scratch,
            compiler_params=pltpu.CompilerParams(vmem_limit_bytes=112 * 1024 * 1024),
            name=name,
        )(A_x.reshape(S, D), A_mem0.reshape(M, D), A_Wq, A_Wk, A_Wv, A_Wo.reshape(H * E, D),
          B_w_in.T, B_w_sp, B_b_sp.reshape(S // 128, 128), B_w_out)
        return out.reshape(B, S, D)

    return fn


pallas_recurrent_scan__memory_aug_recurrent_mem_tr__mixer_gmlp__prompt_kernel = jax.jit(
    build(), static_argnames=("A_seg_len",))
```

```python
import contextlib
import functools
import math

import jax
import jax.numpy as jnp
from jax import lax
import jax.experimental.pallas as pl
import jax.experimental.pallas.tpu as pltpu

F32, BF16, U32 = jnp.float32, jnp.bfloat16, jnp.uint32
NT = (((1,), (1,)), ((), ()))
EPS = 1e-5
LOG2E = math.log2(math.e)

def make_fill(steps):
    pos = {"g": 0, "o": 0, "c": 0}
    fill = {}
    for u, st in enumerate(steps):
        for t, kind, n in st:
            fill.setdefault((u, t), []).append((kind, pos[kind], pos[kind] + n))
            pos[kind] += n
    return fill


DEFAULT_FILL = make_fill([
    [(8, "c", 1), (16, "c", 1), (24, "c", 1), (31, "g", 64), (32, "g", 96), (33, "g", 64), (34, "g", 64), (35, "g", 64)],
    [(8, "c", 1), (16, "c", 1), (31, "g", 64), (32, "g", 96), (33, "g", 64), (34, "g", 64), (35, "g", 64)],
    [(31, "g", 80), (32, "g", 80), (34, "o", 112), (35, "o", 112)],
    [(31, "o", 80), (32, "o", 96), (33, "o", 96), (34, "o", 80), (35, "o", 64)],
])
DEFAULT_CFG = dict(lags=(1, 3, 4), fill=DEFAULT_FILL, c1=144, c2=96, cur=1, lnwhere="first", tie=1, rcp_approx=True, post_norm=True)


def _gelu(x):
    c = math.sqrt(2.0 / math.pi)
    t = jnp.tanh(x * (x * x * (0.044715 * c) + c))
    hx = 0.5 * x
    return hx + hx * t


def _tree_sum(xs):
    xs = list(xs)
    while len(xs) > 1:
        xs = [xs[i] + xs[i + 1] if i + 1 < len(xs) else xs[i] for i in range(0, len(xs), 2)]
    return xs[0]


def _make_kernel(S, D, H, E, M, SEG, FH, cfg):
    L = M + SEG
    TB = 128
    NB = S // TB
    SPB = TB // SEG
    XB = 512
    NXB = S // XB
    KH = S // 2
    HP = H // 2
    lag_s, lag_p, lag_o = cfg["lags"]
    fill = cfg["fill"]
    C1, C2 = cfg["c1"], cfg["c2"]
    FP = -(-FH // 128) * 128
    TPI = -(-FP // 128 // NXB)
    FP2 = TPI * NXB * 128

    def kernel(x_hbm, mem_hbm, wq_hbm, wk_hbm, wv_hbm, wo_hbm, win_hbm, wsp_hbm, bsp_hbm, wout_hbm,
               o_hbm,
               x_v, xo_v, xcur_v, win_u, raw_u, wg_u, wo_u, wspa_v, wspb_v, z1_v, z2_v,
               wout_v, woutt_v, mem_v, bsp_v, bsp_f, y_v, gate_v, s_v,
               sem_x, sem_win, sem_small, sem_grp, sem_spa, sem_wo, sem_spb, sem_out):

        scope = jax.named_scope if cfg.get("scopes") else (lambda n: contextlib.nullcontext())
        CUR = cfg.get("cur", False)
        xin_v = x_v if CUR else xo_v

        def scoped(n, f):
            def g(*a):
                with scope(n):
                    return f(*a)
            return g

        def g_rows(j, r0, n):
            return pl.ds(mult(3 * H * (D // 2) + j * FH + r0, 8), n)

        def w_head(n):
            return pltpu.bitcast(wg_u[n * (D // 2):(n + 1) * (D // 2), :], BF16)

        def when(c):
            return pl.when(c) if not isinstance(c, bool) else (lambda f: f() if c else None)

        def mult(v, n):
            return v if isinstance(v, int) else pl.multiple_of(v, n)

        def cp_x(i):
            rs = [pl.ds(i * XB + t * XB // 2, XB // 2) for t in range(2)]
            return [pltpu.make_async_copy(x_hbm.at[r], xin_v.at[r], sem_x.at[i]) for r in rs]

        def cp_win(half):
            wu = win_hbm.bitcast(U32)
            return [pltpu.make_async_copy(wu.at[pl.ds(half * FH // 2, FH // 2), pl.ds(c * 128, 128)],
                                          win_u.at[half, c], sem_win.at[half]) for c in range(D // 128)]

        cp_xres = None if CUR else pltpu.make_async_copy(x_hbm, x_v, sem_small.at[3])
        cp_mem = pltpu.make_async_copy(mem_hbm, mem_v, sem_small.at[0])
        cp_bsp = pltpu.make_async_copy(bsp_hbm, bsp_v, sem_small.at[1])
        cp_wout = pltpu.make_async_copy(wout_hbm, wout_v.at[pl.ds(0, FH)], sem_small.at[2])

        def cp_group(g):
            cps = []
            for m, w in enumerate((wq_hbm, wk_hbm, wv_hbm)):
                wu = w.bitcast(U32)
                for p in range(HP // NXB):
                    cps.append(pltpu.make_async_copy(
                        wu.at[:, g * (HP // NXB) + p, :], raw_u.at[g, m, p], sem_grp.at[g]))
            r = pl.ds(g * XB, XB)
            cps.append(pltpu.make_async_copy(wsp_hbm.at[r, pl.ds(0, KH)], wspa_v.at[r], sem_spa.at[g]))
            return cps

        def cp_wo(c):
            return pltpu.make_async_copy(wo_hbm.bitcast(U32).at[:, pl.ds(c * 128, 128)], wo_u.at[c], sem_wo.at[0])

        def cp_spb(g):
            r = pl.ds(g * XB, XB)
            return pltpu.make_async_copy(wsp_hbm.at[r, pl.ds(KH, KH)], wspb_v.at[r], sem_spb.at[g])

        def cp_out(j):
            return pltpu.make_async_copy(xo_v.at[pl.ds(mult(S + j * TB, TB), TB)],
                                         o_hbm.at[pl.ds(mult(j * TB, TB), TB)], sem_out.at[0])

        def start(cps):
            for c in cps:
                c.start()

        def wait(cps):
            for c in cps:
                c.wait()

        def stage(i):
            cps = cp_group(i)
            if i + 2 < NXB:
                cps = cp_x(i + 2) + cps
            if i == 0:
                cps = cps + [cp_mem, cp_bsp]
            if i == NXB - 2:
                cps = cps + [cp_wout]
            start(cps)

        start(cp_x(0))

        def ln_rows(r0, n):
            x = xin_v[pl.ds(r0, n), :].astype(F32)
            mu = jnp.sum(x, axis=-1, keepdims=True) * (1.0 / D)
            d = x - mu
            var = jnp.sum(d * d, axis=-1, keepdims=True) * (1.0 / D)
            xf = d * lax.rsqrt(var + EPS)
            xn = xf.astype(BF16)
            xo_v[pl.ds(r0, n), :] = xn
            return xf

        wout_v[FH:FP2, :] = jnp.zeros((FP2 - FH, D), BF16)
        if FP > FH:
            y_v[FH:FP, :] = jnp.zeros((FP - FH, TB), BF16)
        s_v[...] = jnp.zeros(s_v.shape, F32)
        gate_v[...] = jnp.zeros(gate_v.shape, F32)
        with scope("ph_wait_x0"):
            wait(cp_x(0))
        start(cp_win(1) + cp_win(0) + cp_x(1))
        with scope("ph_ln0"):
            for r in range(0, XB, 32):
                ln_rows(r, 32)
            if CUR:
                xcur_v[...] = xo_v[0:XB, :]
        with scope("ph_wait_win"):
            wait(cp_win(1))
            if not cfg.get("midwait"):
                wait(cp_win(0))
        stage(0)

        def win_block(i, carry):
            nxt = i + 1 if isinstance(i, int) else jnp.minimum(i + 1, NXB - 1)
            @when(i + 1 < NXB)
            def _():
                r = pl.ds(mult(nxt * XB, XB), XB)
                pltpu.make_async_copy(x_hbm.at[r], xin_v.at[r], sem_x.at[nxt]).wait()

            for c in range(1, NXB):
                when(i == c - 1)(functools.partial(stage, c))
            NTB = XB // TB

            def load_x(t):
                if CUR:
                    return xcur_v[t * TB:(t + 1) * TB, :]
                return xo_v[pl.ds(mult(i * XB + t * TB, TB), TB), :]

            def zt(half, r0, xb):
                w = jnp.concatenate([pltpu.bitcast(win_u[half, c, r0 // 2:(r0 + C1) // 2, :], BF16)
                                     for c in range(D // 128)], axis=1)
                return _gelu(lax.dot_general(w, xb, NT, preferred_element_type=F32))

            nch = FH // C1
            nv = C1 // 8
            stats = []
            LNR = cfg.get("lnr", 32)
            n_ln = XB // LNR

            def ln_next(n0, tot):
                if not isinstance(nxt, int) or nxt < NXB:
                    for r in range(n0 * n_ln // tot, (n0 + 1) * n_ln // tot):
                        xf = ln_rows(mult(nxt * XB + r * LNR, LNR), LNR)
                        if cfg.get("tie"):
                            if cfg["tie"] == 1:
                                z1_v[jnp.maximum(i, NB + NTB), 0:LNR, :] = xf[:, D - 128:D]
                            else:
                                for cb in range(D // 128):
                                    z1_v[jnp.maximum(i, NB + NTB), cb * LNR:(cb + 1) * LNR, :] = xf[:, cb * 128:(cb + 1) * 128]

            for t in range(NTB):
                means, m2 = [], None
                xb = load_x(t)
                for c in range(nch):
                    z = zt(1, c * C1, xb)
                    z1_v[NB + t, c * C1:(c + 1) * C1, :] = z
                    zs = [z[r:r + 8] for r in range(0, C1, 8)]
                    mean = _tree_sum(zs) * (1.0 / nv)
                    sq = _tree_sum((v - mean) * (v - mean) for v in zs)
                    m2 = sq if m2 is None else m2 + sq
                    means.append(mean)
                    if cfg.get("lnwhere") == "both":
                        ln_next(t * nch + c, 2 * NTB * nch)
                    elif cfg.get("lnwhere") == "first":
                        ln_next(t * nch + c, NTB * nch)
                mu = jnp.sum(_tree_sum(means), axis=0, keepdims=True) * (1.0 / (8 * nch))
                m2 = m2 + nv * _tree_sum((m - mu) * (m - mu) for m in means)
                rs = lax.rsqrt(jnp.sum(m2, axis=0, keepdims=True) * (1.0 / FH) + EPS)
                stats.append((mu, rs))

            if cfg.get("midwait"):
                when(i == 0)(lambda: wait(cp_win(0)))

            raw0 = jnp.maximum(i, NB)
            for t in range(NTB):
                mu, rs = stats[t]
                xb = load_x(t)
                for c in range(nch):
                    z1_v[i * NTB + t, c * C1:(c + 1) * C1, :] = zt(0, c * C1, xb)
                    d = (z1_v[raw0 + t, c * C1:(c + 1) * C1, :] - mu) * rs
                    z2_v[i, c * C1:(c + 1) * C1, t * TB:(t + 1) * TB] = d.astype(BF16)
                    if cfg.get("lnwhere") == "both":
                        ln_next((NTB + t) * nch + c, 2 * NTB * nch)
                    elif cfg.get("lnwhere", "second") == "second":
                        ln_next(t * nch + c, NTB * nch)
                if CUR:
                    xcur_v[t * TB:(t + 1) * TB, :] = xo_v[pl.ds(mult(nxt * XB + t * TB, TB), TB), :]
            return carry

        with scope("ph_A"):
            if cfg.get("unrollA"):
                for i in range(NXB):
                    win_block(i, 0)
            else:
                lax.fori_loop(0, cfg.get('nA', NXB), scoped("ph_Ai", win_block), 0)

        start([cp_wo(c) for c in range(D // 128)] + [cp_spb(g) for g in range(NXB)])
        wait([cp_mem, cp_bsp, cp_wout])

        def pre_block(g, carry):
            rg = pl.ds(mult(g * XB, XB), XB)
            pltpu.make_async_copy(raw_u.at[g], raw_u.at[g], sem_grp.at[g]).wait()
            pltpu.make_async_copy(wspa_v.at[rg], wspa_v.at[rg], sem_spa.at[g]).wait()

            units = [(m, p, r) for m in range(3) for p in range(HP // NXB) for r in range(0, D, 16)]
            nch = FH // C2
            total = nch * (XB // TB)
            done = 0
            for t in range(XB // TB):
                j = g * (XB // TB) + t
                rows = pl.ds(mult(j * TB, TB), TB)
                bias = bsp_f[pl.ds(j, 1), :]
                for c in range(nch):
                    acc = bias
                    for kb in range(KH // XB):
                        lhs = z2_v[kb, c * C2:(c + 1) * C2, :]
                        acc = acc + lax.dot_general(lhs, wspa_v[rows, kb * XB:(kb + 1) * XB], NT,
                                                    preferred_element_type=F32)
                    wg_u[g_rows(j, c * C2, C2), :] = pltpu.bitcast(acc, U32)
                    upto = (t * nch + c + 1) * len(units) // total
                    for m, p, r in units[done:upto]:
                        xe = raw_u[g, m, p, pl.ds(r, 8, stride=2), :]
                        xo = raw_u[g, m, p, pl.ds(r + 1, 8, stride=2), :]
                        h0 = m * H + (g * (HP // NXB) + p) * 2
                        wg_u[pl.ds(mult(h0 * (D // 2) + r // 2, 8), 8), :] = (xe & 0xFFFF) | (xo << 16)
                        wg_u[pl.ds(mult((h0 + 1) * (D // 2) + r // 2, 8), 8), :] = (
                            (xe >> 16) | (xo & jnp.uint32(0xFFFF0000)))
                    done = upto
                if t < TPI:
                    kb = g * TPI + t
                    for cb in range(D // 128):
                        w = wout_v[pl.ds(mult(kb * 128, 128), 128), cb * 128:(cb + 1) * 128].astype(F32)
                        woutt_v[kb, cb * 128:(cb + 1) * 128, :] = w.T.astype(BF16)
            return carry

        bsp_f[...] = bsp_v[...].astype(F32)
        with scope("ph_B"):
            if cfg.get("unrollB"):
                for g in range(NXB):
                    pre_block(g, 0)
            else:
                lax.fori_loop(0, NXB, scoped("ph_Bi", pre_block), 0)

        with scope("ph_wait_wo"):
            wait([cp_wo(c) for c in range(D // 128)] + ([] if CUR else [cp_xres]))

        def combine(j, cb):
            cols = slice(cb * 128, (cb + 1) * 128)
            g = gate_v[cols, :]
            g = (g * pltpu.reciprocal(1.0 + jnp.exp2(g * (-LOG2E)), approx=cfg["rcp_approx"])).T
            x = x_v[pl.ds(mult(j * TB, TB), TB), cols].astype(F32)
            xo_v[pl.ds(mult(S + j * TB, TB), TB), cols] = (x + s_v[j % 2, :, cols] * g).astype(BF16)

        def main_block(j, mem):
            @pl.when(j % (XB // TB) == 0)
            def _():
                gq = j // (XB // TB)
                rg = pl.ds(pl.multiple_of(gq * XB, XB), XB)
                pltpu.make_async_copy(wspb_v.at[rg], wspb_v.at[rg], sem_spb.at[gq]).wait()

            rows = pl.ds(pl.multiple_of(j * TB, TB), TB)

            def filler(kind, r0, r1):
                if kind == "c":
                    combine(jnp.maximum(j - 1, 0), r0)
                elif kind == "g":
                    acc = pltpu.bitcast(wg_u[g_rows(j, r0, r1 - r0), :], F32)
                    for kb in range(KH // XB):
                        lhs = z2_v[KH // XB + kb, r0:r1, :]
                        acc = acc + lax.dot_general(lhs, wspb_v[rows, kb * XB:(kb + 1) * XB], NT,
                                                    preferred_element_type=F32)
                    y = (z1_v[j, r0:r1, :] * acc).astype(BF16)
                    y_v[r0:r1, :] = y
                else:
                    lhs = jnp.concatenate([woutt_v[kb, r0:r1, :]
                                           for kb in range(FP // 128)], axis=1)
                    o = jnp.dot(lhs, y_v[...], preferred_element_type=F32)
                    gate_v[r0:r1, :] = o

            row = lax.broadcasted_iota(jnp.int32, (L, L), 0)
            col = lax.broadcasted_iota(jnp.int32, (L, L), 1)
            mask = (row < M) | (row >= col)

            for u in range(SPB):
                xs = xo_v[pl.ds(mult(j * TB + u * SEG, SEG), SEG), :].astype(F32)
                h = jnp.concatenate([mem, xs], axis=0)
                q, k, v, sc, o = {}, {}, {}, {}, {}
                acc = None
                for t in range(H + lag_o):
                    if t < H:
                        q[t] = jnp.dot(h, w_head(t), preferred_element_type=F32)
                        k[t] = jnp.dot(h, w_head(H + t), preferred_element_type=F32)
                        v[t] = jnp.dot(h, w_head(2 * H + t), preferred_element_type=F32)
                    a = t - lag_s
                    if 0 <= a < H:
                        sc[a] = lax.dot_general(q.pop(a), k.pop(a).astype(BF16), NT, preferred_element_type=F32)
                    a = t - lag_p
                    if 0 <= a < H:
                        s = jnp.where(mask, sc.pop(a) * (E ** -0.5 * LOG2E), -1e9 * LOG2E)
                        e = jnp.exp2(s - jnp.max(s, axis=-1, keepdims=True))
                        r = pltpu.reciprocal(jnp.sum(e, axis=-1, keepdims=True), approx=cfg["rcp_approx"])
                        if cfg["post_norm"]:
                            o[a] = jnp.dot(e, v.pop(a).astype(BF16), preferred_element_type=F32) * r
                        else:
                            o[a] = jnp.dot(e * r, v.pop(a).astype(BF16), preferred_element_type=F32)
                    a = t - lag_o
                    if 0 <= a < H:
                        oo = o.pop(a)
                        r = [jnp.dot(oo, pltpu.bitcast(wo_u[c, a * (E // 2):(a + 1) * (E // 2), :], BF16),
                                     preferred_element_type=F32) for c in range(D // 128)]
                        acc = r if acc is None else [p + n for p, n in zip(acc, r)]
                    for piece in fill.get((u, t), ()):
                        filler(*piece)
                mem = jnp.concatenate([p[0:M] for p in acc], axis=1)
                for c in range(D // 128):
                    s_v[j % 2, u * SEG:(u + 1) * SEG, c * 128:(c + 1) * 128] = acc[c][M:L]

            @pl.when(j > 0)
            def _():
                cp_out(j - 1).start()

            return mem

        with scope("ph_main"):
            lax.fori_loop(0, cfg.get('nM', NB), main_block, mem_v[...].astype(F32))
        for cb in range(D // 128):
            combine(NB - 1, cb)
        cp_out(NB - 1).start()
        nM = cfg.get('nM', NB)
        if nM == NB:
            pltpu.make_async_copy(o_hbm, o_hbm, sem_out.at[0]).wait()
        else:
            for _ in range(max(nM, 1)):
                cp_out(0).wait()
            for gq in range((nM + 3) // 4, NXB):
                cp_spb(gq).wait()

    scratch = [
        pltpu.VMEM((S, D), BF16),
        pltpu.VMEM((2 * S, D), BF16),
        pltpu.VMEM((XB, D), BF16),
        pltpu.VMEM((2, D // 128, FH // 2, 128), U32),
        pltpu.VMEM((NXB, 3, HP // NXB, D, E), U32),
        pltpu.VMEM((3 * H * D // 2 + NB * FH, E), U32),
        pltpu.VMEM((D // 128, H * E // 2, 128), U32),
        pltpu.VMEM((S, KH), BF16),
        pltpu.VMEM((S, KH), BF16),
        pltpu.VMEM((NB + XB // TB + 1, FH, TB), F32),
        pltpu.VMEM((NXB, FH, XB), BF16),
        pltpu.VMEM((FP2, D), BF16),
        pltpu.VMEM((FP2 // 128, D, 128), BF16),
        pltpu.VMEM((M, D), BF16),
        pltpu.VMEM((NB, TB), BF16),
        pltpu.VMEM((NB, TB), F32),
        pltpu.VMEM((FP, TB), BF16),
        pltpu.VMEM((D, TB), F32),
        pltpu.VMEM((2, TB, D), F32),
        pltpu.SemaphoreType.DMA((NXB,)),
        pltpu.SemaphoreType.DMA((2,)),
        pltpu.SemaphoreType.DMA((4,)),
        pltpu.SemaphoreType.DMA((NXB,)),
        pltpu.SemaphoreType.DMA((NXB,)),
        pltpu.SemaphoreType.DMA((1,)),
        pltpu.SemaphoreType.DMA((NXB,)),
        pltpu.SemaphoreType.DMA((1,)),
    ]
    return kernel, scratch


def build(cfg=None, name="rmt_gmlp"):
    cfg = {**DEFAULT_CFG, **(cfg or {})}

    def fn(A_x, A_mem0, A_Wq, A_Wk, A_Wv, A_Wo, A_seg_len, B_x, B_w_in, B_w_sp, B_b_sp, B_w_out):
        B, S, D = A_x.shape
        _, H, E = A_Wq.shape
        M = A_mem0.shape[1]
        FH = B_w_out.shape[0]
        kernel, scratch = _make_kernel(S, D, H, E, M, int(A_seg_len), FH, cfg)
        hbm = pl.BlockSpec(memory_space=pltpu.HBM)
        out = pl.pallas_call(
            kernel,
            out_shape=jax.ShapeDtypeStruct((S, D), A_x.dtype),
            in_specs=[hbm] * 10,
            out_specs=hbm,
            scratch_shapes=scratch,
            compiler_params=pltpu.CompilerParams(vmem_limit_bytes=112 * 1024 * 1024),
            name=name,
        )(A_x.reshape(S, D), A_mem0.reshape(M, D), A_Wq, A_Wk, A_Wv, A_Wo.reshape(H * E, D),
          B_w_in.T, B_w_sp, B_b_sp.reshape(S // 128, 128), B_w_out)
        return out.reshape(B, S, D)

    return fn


pallas_recurrent_scan__memory_aug_recurrent_mem_tr__mixer_gmlp__prompt_kernel = jax.jit(
    build(), static_argnames=("A_seg_len",))
```

```python
import contextlib
import functools
import math

import jax
import jax.numpy as jnp
from jax import lax
import jax.experimental.pallas as pl
import jax.experimental.pallas.tpu as pltpu

F32, BF16, U32 = jnp.float32, jnp.bfloat16, jnp.uint32
NT = (((1,), (1,)), ((), ()))
EPS = 1e-5
LOG2E = math.log2(math.e)

STRASSEN = (
    (((0, 1), (3, 1)), ((0, 1), (3, 1)), ((0, 1), (3, 1))),
    (((3, 1),), ((2, 1), (0, -1)), ((0, 1), (2, 1))),
    (((0, 1), (1, 1)), ((3, 1),), ((0, -1), (1, 1))),
    (((1, 1), (3, -1)), ((2, 1), (3, 1)), ((0, 1),)),
    (((0, 1),), ((1, 1), (3, -1)), ((1, 1), (3, 1))),
    (((2, 1), (3, 1)), ((0, 1),), ((2, 1), (3, -1))),
    (((2, 1), (0, -1)), ((0, 1), (1, 1)), ((3, 1),)),
)


SUMMED = tuple(k for k, (_, b, _) in enumerate(STRASSEN) if len(b) > 1)


def make_fill(steps):
    pos = {}
    fill = {}
    for u, st in enumerate(steps):
        for t, kind, n in st:
            p = pos.get(kind, 0)
            fill.setdefault((u, t), []).append((kind, p, p + n))
            pos[kind] = p + n
    return fill


DEFAULT_FILL = make_fill([
    [(8, "c", 1), (16, "c", 1), (24, "c", 1), (31, "z", 96), (32, "z", 80), (33, "z", 80), (34, "z", 80), (35, "z", 96)],
    [(8, "c", 1), (16, "c", 1), (31, "z", 96), (32, "z", 80), (33, "z", 80), (34, "z", 80), (35, "z", 96)],
    [(31, "o", 64), (32, "o", 64), (33, "o", 64), (34, "o", 64), (35, "o", 80)],
    [(32, "o", 96), (33, "o", 48), (34, "o", 112), (35, "o", 48)],
])
DEFAULT_CFG = dict(lags=(1, 3, 4), lags0=(1, 3, 4), lags3=(1, 3, 4), tail=4, order0=((1, 0), (2,)), fill=DEFAULT_FILL, c1=144, nr=48, rcp_approx=True)


def _gelu2(x):
    c = math.sqrt(2.0 / math.pi)
    return x + x * jnp.tanh(x * (x * x * (0.044715 * c) + c))


def _tree_sum(xs):
    xs = list(xs)
    while len(xs) > 1:
        xs = [xs[i] + xs[i + 1] if i + 1 < len(xs) else xs[i] for i in range(0, len(xs), 2)]
    return xs[0]


def _signed_sum(terms, get):
    (q0, _), *rest = terms
    acc = get(q0)
    for q, sign in rest:
        acc = acc + get(q) if sign > 0 else acc - get(q)
    return acc


def _make_kernel(S, D, H, E, M, SEG, FH, cfg):
    L = M + SEG
    TB = 128
    PB = 2 * TB
    NB = S // TB
    NP = S // PB
    SPB = TB // SEG
    XB = 512
    NXB = S // XB
    NTB = XB // TB
    KH = S // 2
    NMIX = 2 * NXB
    HP = H // 2
    FQ = FH // 2
    DS = D // 256 * 256
    CS = DS // 256
    G0 = 3 * HP * D // 2
    MIX0 = G0 + NP * FH
    MIX1 = MIX0 + 3 * HP * len(SUMMED) * (E // 2)
    WG_ROWS = MIX1 + HP * len(SUMMED) * (E // 2)
    assert CS == 2
    fill = cfg["fill"]
    C1 = cfg["c1"]
    FP = -(-FH // 128) * 128
    TPI = -(-FP // 128 // NMIX)
    FP2 = TPI * NMIX * 128
    HPG = HP // NMIX

    def kernel(x_hbm, mem_hbm, wq_hbm, wk_hbm, wv_hbm, wo_hbm, win_hbm, wsp_hbm, bsp_hbm, wout_hbm,
               o_hbm,
               x_v, xo_v, win_u, raw_u, wg_u, wo_u, wsp_v, wmix0_v, wmix1_v, zraw_v, z2_v,
               wout_v, woutt_v, mem_v, bsp_v, bsp_f, y_v, gate_v, s_v, ahead_v,
               sem_x, sem_win, sem_small, sem_grp, sem_sp, sem_wo, sem_out):

        scope = jax.named_scope if cfg.get("scopes") else (lambda n: contextlib.nullcontext())

        def scoped(n, f):
            def g(*a):
                with scope(n):
                    return f(*a)
            return g

        def mult(v, n):
            return v if isinstance(v, int) else pl.multiple_of(v, n)

        def half(i):
            return slice(i * E, (i + 1) * E)

        def g_rows(p, r0, n):
            return pl.ds(mult(G0 + p * FH + r0, 8), n)

        def w_head(n, d0=0, d1=D):
            return pltpu.bitcast(wg_u[(n // 2 * D + d0) // 2:(n // 2 * D + d1) // 2, half(n % 2)], BF16)

        def qkv_mix_row(m, hp, k):
            return MIX0 + ((m * HP + hp) * len(SUMMED) + SUMMED.index(k)) * (E // 2)

        def wo_mix_row(hp, k):
            return MIX1 + (hp * len(SUMMED) + SUMMED.index(k)) * (E // 2)

        def cp_x(p):
            r = pl.ds(mult(p * PB, PB), PB)
            return pltpu.make_async_copy(x_hbm.at[r], x_v.at[r], sem_x.at[p])

        def cp_win(half):
            wu = win_hbm.bitcast(U32)
            return [pltpu.make_async_copy(wu.at[pl.ds(half * FH // 2, FH // 2), pl.ds(c * 128, 128)],
                                          win_u.at[half, c], sem_win.at[half]) for c in range(D // 128)]

        cp_mem = pltpu.make_async_copy(mem_hbm, mem_v, sem_small.at[0])
        cp_bsp = pltpu.make_async_copy(bsp_hbm, bsp_v, sem_small.at[1])
        cp_wout = pltpu.make_async_copy(wout_hbm, wout_v.at[pl.ds(0, FH)], sem_small.at[2])

        def cp_group(g):
            cps = [pltpu.make_async_copy(wsp_hbm.at[pl.ds(g % NXB * XB, XB), pl.ds(g // NXB * KH, KH)],
                                         wsp_v.at[g], sem_sp.at[g])]
            for m, w in enumerate((wq_hbm, wk_hbm, wv_hbm)):
                wu = w.bitcast(U32)
                for p in range(HPG):
                    cps.append(pltpu.make_async_copy(wu.at[:, g * HPG + p, :], raw_u.at[g, m, p], sem_grp.at[g]))
            return cps + cp_wo(g)

        def cp_wo(g):
            r = pl.ds(mult(g * HPG * E, HPG * E), HPG * E)
            return [pltpu.make_async_copy(wo_hbm.bitcast(U32).at[r, pl.ds(c * 128, 128)], wo_u.at[c, r], sem_wo.at[g])
                    for c in range(D // 128)]

        def cp_out(j):
            return pltpu.make_async_copy(xo_v.at[pl.ds(mult(S + j * TB, TB), TB)],
                                         o_hbm.at[pl.ds(mult(j * TB, TB), TB)], sem_out.at[0])

        def start(cps):
            for c in cps:
                c.start()

        def wait(cps):
            for c in cps:
                c.wait()

        def staged(n_each, stages, body, carry):
            def stage(n, carry):
                for i, cps in enumerate(stages):
                    pl.when(n == i)(lambda: start(cps()))
                return lax.fori_loop(n * n_each, (n + 1) * n_each, body, carry)

            return lax.fori_loop(0, len(stages), stage, carry)

        start([cp_x(0), cp_x(1)] + cp_win(1))

        def ln_rows(r0, n):
            x = x_v[pl.ds(r0, n), :].astype(F32)
            mu = jnp.sum(x, axis=-1, keepdims=True) * (1.0 / D)
            d = x - mu
            var = jnp.sum(d * d, axis=-1, keepdims=True) * (1.0 / D)
            xf = d * lax.rsqrt(var + EPS)
            xo_v[pl.ds(r0, n), :] = xf.astype(BF16)
            return xf

        wout_v[FH:FP2, :] = jnp.zeros((FP2 - FH, D), BF16)
        if FP > FH:
            y_v[FH:FP, :] = jnp.zeros((FP - FH, TB), BF16)
        s_v[...] = jnp.zeros(s_v.shape, F32)
        for t in range(2, 4):
            zraw_v[t] = jnp.zeros((FH, TB), F32)
        gate_v[...] = jnp.zeros(gate_v.shape, F32)
        with scope("ph_start"):
            cp_x(0).wait()
            for r in range(0, PB, 32):
                ln_rows(r, 32)
            wait(cp_win(1))
        start([cp_x(p) for p in range(2, NP)] + [cp_mem, cp_bsp] + cp_group(0) + [cp_wout])

        def z_rows(half, r0, r1, xb):
            w = jnp.concatenate([pltpu.bitcast(win_u[half, c, r0 // 2:r1 // 2, :], BF16)
                                 for c in range(D // 128)], axis=1)
            return _gelu2(lax.dot_general(w, xb, NT, preferred_element_type=F32))

        NR = cfg["nr"]
        UA = cfg.get("ua", 1)

        def z2_operands(p, slot, r, stats):
            quad = []
            for q in range(4):
                mu, rs = stats[q % 2]
                r0 = r + (q // 2) * FQ
                z = zraw_v[2 * slot + q % 2, r0:r0 + NR, :].reshape(NR // 8, 8, TB)
                quad.append(((z - mu) * rs).reshape(NR, TB))
            for k, (a_terms, _, _) in enumerate(STRASSEN):
                z2_v[p, k, r:r + NR, :] = _signed_sum(a_terms, quad.__getitem__).astype(BF16)

        def z2_pair(p, prev_moments):
            nxt = jnp.minimum(p + 1, NP - 1)
            prev_stats = z2_stats(prev_moments)
            moments = []
            nch = FH // C1
            nv = C1 // 8
            n_ln = PB // 32
            n_op = FQ // NR
            xbs = [xo_v[pl.ds(mult(p * PB + t * TB, TB), TB), :] for t in range(2)]
            for t in range(2):
                means, m2 = [], None
                for c in range(nch):
                    z = z_rows(1, c * C1, (c + 1) * C1, xbs[t])
                    zraw_v[2 * (p % 2) + t, c * C1:(c + 1) * C1, :] = z
                    zs = [z[r:r + 8] for r in range(0, C1, 8)]
                    mean = _tree_sum(zs) * (1.0 / nv)
                    sq = _tree_sum((v - mean) * (v - mean) for v in zs)
                    m2 = sq if m2 is None else m2 + sq
                    means.append(mean)
                    n0 = t * nch + c
                    for r in range(n0 * n_ln // (2 * nch), (n0 + 1) * n_ln // (2 * nch)):
                        xf = ln_rows(mult(nxt * PB + r * 32, 32), 32)
                        zraw_v[jnp.maximum(p % 2, 4), 0:32, :] = xf[:, D - 128:D]
                    for r in range(n0 * n_op // (2 * nch), (n0 + 1) * n_op // (2 * nch)):
                        z2_operands(jnp.maximum(p - 1, 0), 1 - p % 2, r * NR, prev_stats)
                moments.append((tuple(means), m2))
            return tuple(moments)

        def z2_stats(moments):
            stats = []
            for means, m2 in moments:
                mu = jnp.sum(_tree_sum(means), axis=0, keepdims=True) * (1.0 / (8 * len(means)))
                m2 = m2 + (C1 // 8) * _tree_sum((m - mu) * (m - mu) for m in means)
                rs = lax.rsqrt(jnp.sum(m2, axis=0, keepdims=True) * (1.0 / FH) + 4 * EPS)
                stats.append((jnp.broadcast_to(mu, (8, TB)), jnp.broadcast_to(rs, (8, TB))))
            return stats

        def z2_block(n, moments):
            for p in range(UA):
                pl.when(n * UA + p + 1 < NP)(lambda: cp_x(jnp.minimum(n * UA + p + 1, NP - 1)).wait())
            for p in range(UA):
                moments = z2_pair(n * UA + p, moments)
            return moments

        zero_row = jnp.zeros((8, TB), F32)
        with scope("ph_A"):
            moments = staged(NP // 2 // UA, [lambda: [], lambda: cp_group(1)],
                             scoped("ph_Ai", z2_block), (((zero_row,) * (FH // C1), zero_row),) * 2)
        stats = z2_stats(moments)
        start(cp_group(2))
        for r in range(0, FQ, NR):
            z2_operands(NP - 1, (NP - 1) % 2, r, stats)

        MR = cfg.get("mr", 16)
        MN = cfg.get("mn", 1)
        pieces = [(r, n) for r in range(0, TB, MR) for n in range(0, KH // PB, MN)]

        def mix_piece(g, slot, r, n0):
            for n in range(n0, n0 + MN):
                quad = []
                for q in range(4):
                    r0, c0 = slot * PB + (q % 2) * TB + r, (2 * n + q // 2) * TB
                    quad.append(wsp_v[g, r0:r0 + MR, c0:c0 + TB])
                wide = [w.astype(F32) for w in quad]
                for k, (_, b_terms, _) in enumerate(STRASSEN):
                    if len(b_terms) > 1:
                        w = _signed_sum(b_terms, wide.__getitem__).astype(BF16)
                    else:
                        w = quad[b_terms[0][0]]
                    (wmix0_v, wmix1_v)[slot][k, n, r:r + MR, :] = w

        def mix_product(b0, slot, k, r0, r1):
            lhs = jnp.concatenate([z2_v[b0 + b, k, r0:r1, :] for b in range(KH // PB)], axis=1)
            rhs = jnp.concatenate([(wmix0_v, wmix1_v)[slot][k, b] for b in range(KH // PB)], axis=1)
            return lax.dot_general(lhs, rhs, NT, preferred_element_type=F32)

        def mix_accumulate(acc, k, prod, first, last):
            for q, sign in STRASSEN[k][2]:
                base = acc[q] if q in acc else first(q)
                acc[q] = base + prod if sign > 0 else base - prod
                if all(q != q2 for _, _, cs in STRASSEN[k + 1:] for q2, _ in cs):
                    last(q, acc.pop(q))

        wait([cp_mem, cp_bsp, cp_wout])
        bsp_f[...] = bsp_v[...].astype(F32)
        pltpu.make_async_copy(wsp_v.at[0], wsp_v.at[0], sem_sp.at[0]).wait()
        for r, n in pieces:
            mix_piece(0, 0, r, n)

        def mix_block(g, carry):
            nxt = jnp.minimum(g + 1, NMIX - 1)
            GCH = cfg.get("gch", (96, 96, 80, 80, 80))
            nch = len(GCH)

            def split_heads(m, p, r):
                xe = raw_u[g, m, p, pl.ds(r, 16, stride=2), :]
                xo = raw_u[g, m, p, pl.ds(r + 1, 16, stride=2), :]
                words = (xe & 0xFFFF) | (xo << 16), (xe >> 16) | (xo & jnp.uint32(0xFFFF0000))
                for i, w in enumerate(words):
                    wg_u[pl.ds(mult((m * HP + g * HPG + p) * (D // 2) + r // 2, 8), 16), half(i)] = w
                return words

            def store_sums(words, row, c):
                wide = [pltpu.bitcast(w, BF16).astype(F32) for w in words]
                for k in SUMMED:
                    w = _signed_sum(STRASSEN[k][1], wide.__getitem__).astype(BF16)
                    wg_u[pl.ds(mult(row(k), 8), 16), half(c)] = pltpu.bitcast(w, U32)

            def qkv_unit(m, p, r):
                if r >= DS:
                    split_heads(m, p, r)
                else:
                    store_sums(split_heads(m, p, r) + split_heads(m, p, r + DS // 2),
                               lambda k: qkv_mix_row(m, g * HPG + p, k) + r % E // 2, r // E)

            def wo_unit(p, c, r):
                hp = g * HPG + p
                words = [wo_u[(q % 2) * CS + c, pl.ds(mult((2 * hp + q // 2) * (E // 2) + r, 8), 16), :]
                         for q in range(4)]
                store_sums(words, lambda k: wo_mix_row(hp, k) + r, c)

            units = [functools.partial(qkv_unit, m, p, r) for m in range(3) for p in range(HPG)
                     for r in (*range(0, DS // 2, 32), *range(DS, D, 32))]
            units += [functools.partial(wo_unit, p, c, r) for p in range(HPG) for c in range(CS)
                      for r in range(0, E // 2, 16)]
            total = nch * (XB // PB) * 4
            count = [0, 0]

            def relayout():
                count[0] += 1
                upto = count[0] * len(units) // total
                for unit in units[count[1]:upto]:
                    unit()
                count[1] = upto

            for t in range(XB // PB):
                j = g % NXB * (XB // PB) + t
                count[2:] = [0, 0]
                bias = [bsp_f[pl.ds(2 * j + n, 1), :] for n in range(2)]
                for c in range(nch):
                    def rows(q):
                        return g_rows(j, (q // 2) * FQ + sum(GCH[:c]), GCH[c])

                    def first(q):
                        return jnp.where(g >= NXB, pltpu.bitcast(wg_u[rows(q), half(q % 2)], F32), bias[q % 2])

                    def last(q, val):
                        wg_u[rows(q), half(q % 2)] = pltpu.bitcast(val, U32)
                        relayout()
                        count[2] += 1
                        upto = count[2] * len(pieces) // (4 * nch)
                        if upto > count[3] and t in cfg.get("mixtie", (0, 1)):
                            wsp_v[jnp.maximum(g, NMIX), 0:16, 0:TB] = val[0:16].astype(BF16)
                        for r, n in pieces[count[3]:upto]:
                            mix_piece(g if t == 0 else nxt, 1 - t, r, n)
                        count[3] = upto

                    acc = {}
                    for k in range(7):
                        mix_accumulate(acc, k, mix_product(g // NXB * (KH // PB), t, k, sum(GCH[:c]), sum(GCH[:c + 1])),
                                       first, last)
                for n in range(t * TPI // (XB // PB), (t + 1) * TPI // (XB // PB)):
                    kb = g * TPI + n
                    for cb in range(D // 128):
                        w = wout_v[pl.ds(mult(kb * 128, 128), 128), cb * 128:(cb + 1) * 128].astype(F32)
                        woutt_v[kb, cb * 128:(cb + 1) * 128, :] = w.T.astype(BF16)
            return carry

        UB = cfg.get("ub", 1)

        def mix_blocks(n, carry):
            for i in range(UB):
                g = n * UB + i
                nxt = jnp.minimum(g + 1, NMIX - 1)
                pltpu.make_async_copy(raw_u.at[g], raw_u.at[g], sem_grp.at[g]).wait()
                wait(cp_wo(g))
                pl.when(g + 1 < NMIX)(
                    lambda: pltpu.make_async_copy(wsp_v.at[nxt], wsp_v.at[nxt], sem_sp.at[nxt]).wait())
            for i in range(UB):
                mix_block(n * UB + i, carry)
            return carry

        with scope("ph_B"):
            staged(1, [functools.partial(cp_group, g) for g in range(3, NMIX)] + [lambda: cp_win(0)] + [list] * 2,
                   scoped("ph_Bi", mix_blocks), 0)

        with scope("ph_wait_wo"):
            wait(cp_win(0))

        def combine(j, cb):
            cols = slice(cb * 128, (cb + 1) * 128)
            g = gate_v[cols, :]
            g = (g * pltpu.reciprocal(1.0 + jnp.exp2(g * (-LOG2E)), approx=cfg["rcp_approx"])).T
            x = x_v[pl.ds(mult(j * TB, TB), TB), cols].astype(F32)
            xo_v[pl.ds(mult(S + j * TB, TB), TB), cols] = (x + s_v[j % 2, :, cols] * g).astype(BF16)

        def main_block(j, mem):
            xb = xo_v[pl.ds(mult(j * TB, TB), TB), :]

            def filler(kind, r0, r1):
                if kind == "c":
                    for cb in range(r0, r1):
                        combine(jnp.maximum(j - 1, 0), cb)
                elif kind == "z":
                    g2 = pltpu.bitcast(wg_u[g_rows(j // 2, r0, r1 - r0), :], F32)
                    g = jnp.where(j % 2 == 0, g2[:, half(0)], g2[:, half(1)])
                    y_v[r0:r1, :] = (z_rows(0, r0, r1, xb) * (0.5 * g)).astype(BF16)
                else:
                    lhs = jnp.concatenate([woutt_v[kb, r0:r1, :] for kb in range(FP // 128)], axis=1)
                    gate_v[r0:r1, :] = jnp.dot(lhs, y_v[...], preferred_element_type=F32)

            row = lax.broadcasted_iota(jnp.int32, (L, L), 0)
            col = lax.broadcasted_iota(jnp.int32, (L, L), 1)
            mask = (row < M) | (row >= col)

            def dot(a, b):
                return jnp.dot(a, b, preferred_element_type=F32)

            def wo(hd, c):
                return pltpu.bitcast(wo_u[c, hd * (E // 2):(hd + 1) * (E // 2), :], BF16)

            zero = jnp.minimum(j, 0)
            NT_ROWS = SEG - M

            def put(slot, rows):
                if rows.shape[0]:
                    ahead_v[zero + slot, 0:rows.shape[0], :] = rows

            def get(slot, n):
                return [ahead_v[zero + slot, 0:n, :]] if n else []

            for u in range(SPB):
                r0 = 0 if u == 0 else SEG + u * NT_ROWS
                r1 = SEG + (u + 1) * NT_ROWS
                lo, hi = r0 // 16 * 16, -(-r1 // 16) * 16
                xs = xo_v[pl.ds(mult(j * TB + lo, 16), hi - lo), :].astype(F32)[r0 - lo:r1 - lo]
                h = jnp.concatenate([mem, xs], axis=0)
                if u == 0:
                    quad = [h[(q // 2) * SEG:(q // 2 + 1) * SEG, (q % 2) * DS // 2:(q % 2 + 1) * DS // 2]
                            for q in range(4)]
                    h_ops = [_signed_sum(a_terms, quad.__getitem__) for a_terms, _, _ in STRASSEN]
                n_wait = r0 - u * SEG
                qkv, sc, o = {}, {}, {}
                acc = {}

                def keep(m, hd, rows):
                    new = SEG - n_wait
                    qkv[m, hd] = jnp.concatenate(
                        [rows[0:M]] + get(3 * hd + m, n_wait) + [rows[M:M + new]], axis=0)
                    if M + new < rows.shape[0]:
                        put(3 * hd + m, rows[M + new:])

                def project_pair(m, hp):
                    tail = [dot(h[:, DS:D], w_head(m * H + 2 * hp + i, DS, D)) for i in range(2)]
                    c, out = {}, {}
                    for k, (_, b_terms, _) in enumerate(STRASSEN):
                        if k in SUMMED:
                            w = jnp.concatenate([pltpu.bitcast(wg_u[pl.ds(qkv_mix_row(m, hp, k), E // 2), half(c)], BF16)
                                                 for c in range(CS)], axis=0)
                        else:
                            q = b_terms[0][0]
                            w = w_head(m * H + 2 * hp + q % 2, (q // 2) * DS // 2, (q // 2 + 1) * DS // 2)
                        mix_accumulate(c, k, dot(h_ops[k], w),
                                       lambda q: tail[q % 2][(q // 2) * SEG:(q // 2 + 1) * SEG], out.__setitem__)
                    for i in range(2):
                        keep(m, 2 * hp + i, jnp.concatenate([out[i], out[2 + i]], axis=0))

                def add(key, val):
                    acc[key] = acc[key] + val if key in acc else val

                def out_rows(hd):
                    rows = o.pop(hd)
                    n_old = u * M
                    new = (2 * SEG if u == SPB - 1 else SEG) - M - n_old
                    lhs = jnp.concatenate([rows[0:M]] + get(3 * H + hd, n_old) + [rows[M:M + new]], axis=0)
                    if M + new < L:
                        put(3 * H + hd, rows[M + new:])
                    return lhs

                def out_pair(hp):
                    lhs = [out_rows(2 * hp + i) for i in range(2)]
                    quad = [lhs[q % 2][(q // 2) * SEG:(q // 2 + 1) * SEG] for q in range(4)]
                    for i in range(2):
                        for c in range(2 * CS, D // 128):
                            add(c, dot(lhs[i], wo(2 * hp + i, c)))
                    for k, (a_terms, b_terms, _) in enumerate(STRASSEN):
                        a_op = _signed_sum(a_terms, quad.__getitem__)
                        for c in range(CS):
                            if k in SUMMED:
                                w = pltpu.bitcast(wg_u[pl.ds(wo_mix_row(hp, k), E // 2), half(c)], BF16)
                            else:
                                q = b_terms[0][0]
                                w = wo(2 * hp + q // 2, (q % 2) * CS + c)
                            add((k, c), dot(a_op, w))

                lag_s, lag_p, lag_o = cfg["lags0"] if u == 0 else cfg["lags3"] if u == SPB - 1 else cfg["lags"]
                for t in range(H + max(lag_o, cfg["tail"])):
                    if t < H:
                        if u > 0:
                            for m in range(3):
                                keep(m, t, dot(h, w_head(m * H + t)))
                        else:
                            for m in cfg["order0"][t % 2]:
                                project_pair(m, t // 2)
                    a = t - lag_s
                    if 0 <= a < H:
                        sc[a] = lax.dot_general(qkv.pop((0, a)), qkv.pop((1, a)).astype(BF16), NT,
                                                preferred_element_type=F32)
                    a = t - lag_p
                    if 0 <= a < H:
                        s = jnp.where(mask, sc.pop(a) * (E ** -0.5 * LOG2E), -1e9 * LOG2E)
                        e = jnp.exp2(s - jnp.max(s, axis=-1, keepdims=True))
                        r = pltpu.reciprocal(jnp.sum(e, axis=-1, keepdims=True), approx=cfg["rcp_approx"])
                        o[a] = dot(e, qkv.pop((2, a)).astype(BF16)) * r
                    a = t - lag_o
                    if 0 <= a < H:
                        if u < SPB - 1:
                            lhs = out_rows(a)
                            for c in range(D // 128):
                                add(c, dot(lhs, wo(a, c)))
                        elif a % 2:
                            out_pair(a // 2)
                    for piece in fill.get((u, t), ()):
                        filler(*piece)
                if u == SPB - 1:
                    for c in range(CS):
                        part, out = {}, {}
                        for k, (_, _, c_terms) in enumerate(STRASSEN):
                            for q, sign in c_terms:
                                prod = acc[k, c]
                                out[q] = (prod if q not in out else out[q] + prod if sign > 0 else out[q] - prod)
                        for i in range(2):
                            acc[i * CS + c] = jnp.concatenate([out[i], out[2 + i]], axis=0)
                mem = jnp.concatenate([acc[c][0:M] for c in range(D // 128)], axis=1)
                for c in range(D // 128):
                    s_v[j % 2, u * NT_ROWS:u * NT_ROWS + acc[c].shape[0] - M, c * 128:(c + 1) * 128] = acc[c][M:]

            @pl.when(j > 0)
            def _():
                cp_out(j - 1).start()

            return mem

        with scope("ph_main"):
            lax.fori_loop(0, NB, main_block, mem_v[...].astype(F32))
        for cb in range(D // 128):
            combine(NB - 1, cb)
        cp_out(NB - 1).start()
        pltpu.make_async_copy(o_hbm, o_hbm, sem_out.at[0]).wait()

    scratch = [
        pltpu.VMEM((S, D), BF16),
        pltpu.VMEM((2 * S, D), BF16),
        pltpu.VMEM((2, D // 128, FH // 2, 128), U32),
        pltpu.VMEM((NMIX, 3, HPG, D, E), U32),
        pltpu.VMEM((WG_ROWS, 2 * E), U32),
        pltpu.VMEM((D // 128, H * E // 2, 128), U32),
        pltpu.VMEM((NMIX + 1, XB, KH), BF16),
        pltpu.VMEM((7, KH // PB, TB, TB), BF16),
        pltpu.VMEM((7, KH // PB, TB, TB), BF16),
        pltpu.VMEM((5, FH, TB), F32),
        pltpu.VMEM((NP, 7, FQ, TB), BF16),
        pltpu.VMEM((FP2, D), BF16),
        pltpu.VMEM((FP2 // 128, D, 128), BF16),
        pltpu.VMEM((M, D), BF16),
        pltpu.VMEM((NB, TB), BF16),
        pltpu.VMEM((NB, TB), F32),
        pltpu.VMEM((FP, TB), BF16),
        pltpu.VMEM((D, TB), F32),
        pltpu.VMEM((2, TB, D), F32),
        pltpu.VMEM((4 * H, SEG - M, E), F32),
        pltpu.SemaphoreType.DMA((NP,)),
        pltpu.SemaphoreType.DMA((2,)),
        pltpu.SemaphoreType.DMA((3,)),
        pltpu.SemaphoreType.DMA((NMIX,)),
        pltpu.SemaphoreType.DMA((NMIX,)),
        pltpu.SemaphoreType.DMA((NMIX,)),
        pltpu.SemaphoreType.DMA((1,)),
    ]
    return kernel, scratch


def build(cfg=None, name="rmt_gmlp"):
    cfg = {**DEFAULT_CFG, **(cfg or {})}

    def fn(A_x, A_mem0, A_Wq, A_Wk, A_Wv, A_Wo, A_seg_len, B_x, B_w_in, B_w_sp, B_b_sp, B_w_out):
        B, S, D = A_x.shape
        _, H, E = A_Wq.shape
        M = A_mem0.shape[1]
        FH = B_w_out.shape[0]
        kernel, scratch = _make_kernel(S, D, H, E, M, int(A_seg_len), FH, cfg)
        hbm = pl.BlockSpec(memory_space=pltpu.HBM)
        out = pl.pallas_call(
            kernel,
            out_shape=jax.ShapeDtypeStruct((S, D), A_x.dtype),
            in_specs=[hbm] * 10,
            out_specs=hbm,
            scratch_shapes=scratch,
            compiler_params=pltpu.CompilerParams(vmem_limit_bytes=120 * 1024 * 1024),
            name=name,
        )(A_x.reshape(S, D), A_mem0.reshape(M, D), A_Wq, A_Wk, A_Wv, A_Wo.reshape(H * E, D),
          B_w_in.T, B_w_sp, B_b_sp.reshape(S // 128, 128), B_w_out)
        return out.reshape(B, S, D)

    return fn


pallas_recurrent_scan__memory_aug_recurrent_mem_tr__mixer_gmlp__prompt_kernel = jax.jit(
    build(), static_argnames=("A_seg_len",))
```

```python
import contextlib
import functools
import math

import jax
import jax.numpy as jnp
from jax import lax
import jax.experimental.pallas as pl
import jax.experimental.pallas.tpu as pltpu

F32, BF16, U32 = jnp.float32, jnp.bfloat16, jnp.uint32
LANES = 128
EPS = 1e-5
LOG2E = math.log2(math.e)

STRASSEN = (
    (((0, 1), (3, 1)), ((0, 1), (3, 1)), ((0, 1), (3, 1))),
    (((3, 1),), ((2, 1), (0, -1)), ((0, 1), (2, 1))),
    (((0, 1), (1, 1)), ((3, 1),), ((0, -1), (1, 1))),
    (((1, 1), (3, -1)), ((2, 1), (3, 1)), ((0, 1),)),
    (((0, 1),), ((1, 1), (3, -1)), ((1, 1), (3, 1))),
    (((2, 1), (3, 1)), ((0, 1),), ((2, 1), (3, -1))),
    (((2, 1), (0, -1)), ((0, 1), (1, 1)), ((3, 1),)),
)
SUMMED = tuple(k for k, (_, b_terms, _) in enumerate(STRASSEN) if len(b_terms) > 1)

LAG_SCORES, LAG_VALUES, LAG_OUT = 1, 3, 4


def _lay_out(steps):
    end, plan = {}, {}
    for u, pieces in enumerate(steps):
        for slot, kind, size in pieces:
            start = end.get(kind, 0)
            end[kind] = start + size
            plan.setdefault((u, slot), []).append((kind, start, start + size))
    return plan, end


SIDE_WORK = (
    ((8, "out", 1), (16, "out", 1),
     (31, "z1", 96), (32, "z1", 80), (33, "z1", 80), (34, "z1", 64), (35, "z1", 112)),
    ((6, "out", 1), (14, "out", 1), (22, "out", 1),
     (31, "z1", 96), (32, "z1", 64), (33, "z1", 112), (34, "z1", 80), (35, "z1", 80)),
    ((31, "w_out", 64), (32, "w_out", 64), (33, "w_out", 64), (34, "w_out", 64), (35, "w_out", 80)),
    ((32, "w_out", 96), (33, "w_out", 48), (34, "w_out", 112), (35, "w_out", 48)),
)
Z2_ROWS = 144
MIX_ROWS = ((80, 80, 80, 96, 96), (96, 96, 80, 80, 80))


def _dot(a, b):
    return jnp.dot(a, b, preferred_element_type=F32)


def _dot_nt(a, b):
    return lax.dot_general(a, b, (((1,), (1,)), ((), ())), preferred_element_type=F32)


def _twice_gelu(x):
    c = math.sqrt(2.0 / math.pi)
    return x + x * jnp.tanh(x * (x * x * (0.044715 * c) + c))


def _reciprocal(x):
    r = pltpu.reciprocal(x, approx=True)
    return r * (2.0 - x * r)


def _tree_sum(xs):
    xs = list(xs)
    while len(xs) > 1:
        xs = [xs[i] + xs[i + 1] if i + 1 < len(xs) else xs[i] for i in range(0, len(xs), 2)]
    return xs[0]


def _signed_sum(terms, blocks):
    (first, _), *rest = terms
    total = blocks[first]
    for q, sign in rest:
        total = total + blocks[q] if sign > 0 else total - blocks[q]
    return total


def _accumulate(sums, key, value, sign=1):
    if key in sums:
        sums[key] = sums[key] + value if sign > 0 else sums[key] - value
    else:
        sums[key] = value if sign > 0 else -value


def _aligned(start, size, unit):
    return pl.ds(start if isinstance(start, int) else pl.multiple_of(start, unit), size)


def _tile(i):
    return slice(i * LANES, (i + 1) * LANES)


def _start(copies):
    for c in copies:
        c.start()


def _wait(copies):
    for c in copies:
        c.wait()


def _make_kernel(S, D, H, M, SEG, FH, cfg):
    E = TB = LANES
    PB = 2 * TB
    NB, NP = S // TB, S // PB
    SPB = TB // SEG
    DT = D // LANES
    DS = D // PB * PB
    CS = DS // PB
    FQ = FH // 2
    FT = -(-FH // LANES)
    FP = -(-FH // PB) * PB
    KH = S // 2
    NG = NP // 2
    HP = H // 2
    HG = HP // (2 * NG)
    NW = FP // PB * DT
    WG = -(-NW // (2 * NG))
    NSUM = len(SUMMED) * E // 2
    ROW_G = 3 * HP * D // 2
    ROW_SUM = ROW_G + NP * FH
    ROWS = ROW_SUM + 4 * HP * NSUM
    side_work, side_total = _lay_out(cfg.get("side", SIDE_WORK))
    mix_rows = cfg.get("mix_rows", MIX_ROWS)
    assert side_total == {"out": DT, "z1": FH, "w_out": D} and all(sum(r) == FQ for r in mix_rows)
    assert CS == 2 and SPB == 4 and SEG == SPB * M and FQ % Z2_ROWS == 0 and HP == 2 * NG * HG

    def kernel(x_hbm, mem_hbm, wq_hbm, wk_hbm, wv_hbm, wo_hbm, win_hbm, wsp_hbm, bsp_hbm, wout_hbm,
               o_hbm,
               x_v, xo_v, win_u, raw_u, big_u, wo_u, wsp_v, wmix0_v, wmix1_v, zraw_v, z2_v,
               wout_v, woutt_v, mem_v, bsp_v, bias_v, y_v, gate_v, s_v, ahead_v,
               sem_x, sem_win, sem_small, sem_raw, sem_sp, sem_wo, sem_out):
        scope = jax.named_scope if cfg.get("scopes") else (lambda name: contextlib.nullcontext())

        def scoped(name, f):
            def g(*args):
                with scope(name):
                    return f(*args)
            return g

        def w_head(n, d0=0, d1=D):
            return pltpu.bitcast(big_u[(n // 2 * D + d0) // 2:(n // 2 * D + d1) // 2, _tile(n % 2)], BF16)

        def w_sum(m, hp, k, c):
            row = ROW_SUM + (m * HP + hp) * NSUM + SUMMED.index(k) * E // 2
            return pltpu.bitcast(big_u[row:row + E // 2, _tile(c)], BF16)

        def wo_head(hd, c):
            return pltpu.bitcast(wo_u[c, hd * E // 2:(hd + 1) * E // 2, :], BF16)

        def cp_x(p):
            rows = _aligned(p * PB, PB, PB)
            return pltpu.make_async_copy(x_hbm.at[rows], x_v.at[rows], sem_x.at[p])

        def cp_win(half, part=0, parts=1):
            n = FH // 2 // parts
            return [pltpu.make_async_copy(
                win_hbm.bitcast(U32).at[pl.ds(half * FH // 2 + part * n, n), pl.ds(c * LANES, LANES)],
                win_u.at[half, c, pl.ds(part * n, n)], sem_win.at[half + part]) for c in range(DT)]

        def cp_small():
            return [pltpu.make_async_copy(mem_hbm, mem_v, sem_small.at[0]),
                    pltpu.make_async_copy(bsp_hbm, bsp_v, sem_small.at[1]),
                    pltpu.make_async_copy(wout_hbm, wout_v.at[pl.ds(0, FH)], sem_small.at[2])]

        def cp_wo(g):
            rows = _aligned(g * HG * E, HG * E, HG * E)
            return [pltpu.make_async_copy(wo_hbm.bitcast(U32).at[rows, pl.ds(c * LANES, LANES)],
                                          wo_u.at[c, rows], sem_wo.at[g]) for c in range(DT)]

        def cp_group(g):
            copies = [pltpu.make_async_copy(
                wsp_hbm.at[pl.ds(g % NG * 2 * PB, 2 * PB), pl.ds(g // NG * KH, KH)], wsp_v.at[g], sem_sp.at[g])]
            for m, w_hbm in enumerate((wq_hbm, wk_hbm, wv_hbm)):
                copies += [pltpu.make_async_copy(w_hbm.bitcast(U32).at[:, g, p, :], raw_u.at[g, m, p], sem_raw.at[g])
                           for p in range(HG)]
            return copies + cp_wo(g)

        def wait_filled(buf, sem):
            pltpu.make_async_copy(buf, buf, sem).wait()

        def layernorm_rows(r0, n):
            rows = _aligned(r0, n, n)
            x = x_v[rows, :].astype(F32)
            d = x - jnp.sum(x, axis=-1, keepdims=True) * (1.0 / D)
            xn = d * lax.rsqrt(jnp.sum(d * d, axis=-1, keepdims=True) * (1.0 / D) + EPS)
            xo_v[rows, :] = xn.astype(BF16)
            return xn

        def z_rows(half, r0, r1, xn):
            w = jnp.concatenate([pltpu.bitcast(win_u[half, c, r0 // 2:r1 // 2, :], BF16) for c in range(DT)], axis=1)
            return _twice_gelu(_dot_nt(w, xn))

        def z2_stats(moments):
            stats = []
            for means, m2 in moments:
                mu = jnp.sum(_tree_sum(means), axis=0, keepdims=True) * (1.0 / (8 * len(means)))
                m2 = m2 + (Z2_ROWS // 8) * _tree_sum((m - mu) * (m - mu) for m in means)
                rs = lax.rsqrt(jnp.sum(m2, axis=0, keepdims=True) * (1.0 / FH) + 4 * EPS)
                stats.append((jnp.broadcast_to(mu, (8, TB)), jnp.broadcast_to(rs, (8, TB))))
            return stats

        def z2_operands(p, slot, r, stats):
            quad = []
            for q in range(4):
                mu, rs = stats[q % 2]
                r0 = r + q // 2 * FQ
                z = zraw_v[2 * slot + q % 2, r0:r0 + Z2_ROWS, :].reshape(Z2_ROWS // 8, 8, TB)
                quad.append(((z - mu) * rs).reshape(Z2_ROWS, TB))
            for k, (a_terms, _, _) in enumerate(STRASSEN):
                z2_v[p, k, r:r + Z2_ROWS, :] = _signed_sum(a_terms, quad).astype(BF16)

        def z2_pair(p, prev_moments):
            opening = prev_moments is None
            nxt = p + 1 if opening else jnp.minimum(p + 1, NP - 1)
            prev_stats = None if opening else z2_stats(prev_moments)
            xn = [xo_v[_aligned(p * PB + t * TB, TB, TB), :] for t in range(2)]
            order = [(t, r) for t in range(2) for r in range(0, FH, Z2_ROWS)]
            if opening:
                order.sort(key=lambda tr: tr[1])
            steps, n_norm, n_ops = len(order), PB // 64, FQ // Z2_ROWS
            means, m2 = ([], []), {}
            for n, (t, r) in enumerate(order):
                if opening and n == 0:
                    _wait(cp_win(1, 0, 2))
                if opening and n == steps // 2:
                    _wait(cp_win(1, 1, 2) + [cp_x(1)])
                    _start([cp_x(i) for i in range(2, NP)] + cp_small())
                z = z_rows(1, r, r + Z2_ROWS, xn[t])
                zraw_v[2 * (p % 2) + t, r:r + Z2_ROWS, :] = z
                parts = [z[i:i + 8] for i in range(0, Z2_ROWS, 8)]
                mean = _tree_sum(parts) * (1.0 / len(parts))
                _accumulate(m2, t, _tree_sum((v - mean) * (v - mean) for v in parts))
                means[t].append(mean)
                if opening:
                    late = max(0, n + 1 - steps // 2)
                    for i in range(max(0, late - 1) * n_norm // (steps // 2), late * n_norm // (steps // 2)):
                        layernorm_rows(nxt * PB + i * 64, 64)
                    continue
                for i in range(n * n_norm // steps, (n + 1) * n_norm // steps):
                    rows = layernorm_rows(nxt * PB + i * 64, 64)
                    zraw_v[jnp.maximum(p % 2, 4), 0:64, :] = rows[:, D - LANES:D]
                for i in range(n * n_ops // steps, (n + 1) * n_ops // steps):
                    z2_operands(p - 1, 1 - p % 2, i * Z2_ROWS, prev_stats)
            return tuple((tuple(means[t]), m2[t]) for t in range(2))

        def z2_step(p, moments):
            pl.when(p + 1 < NP)(lambda: cp_x(jnp.minimum(p + 1, NP - 1)).wait())
            for g in (1, 2):
                pl.when(p == 3 * g)(lambda: _start(cp_group(g)))
            return z2_pair(p, moments)

        _start([cp_x(0)] + cp_win(1, 0, 2))
        wout_v[FH:FP, :] = jnp.zeros((FP - FH, D), BF16)
        y_v[FH:FT * LANES, :] = jnp.zeros((FT * LANES - FH, TB), BF16)
        s_v[...] = jnp.zeros(s_v.shape, F32)
        gate_v[...] = jnp.zeros(gate_v.shape, F32)
        with scope("ph_start"):
            cp_x(0).wait()
            _start(cp_win(1, 1, 2) + [cp_x(1)])
            for r in range(0, PB, 32):
                layernorm_rows(r, 32)
        with scope("ph_A0"):
            moments = z2_pair(0, None)
        _start(cp_group(0))
        with scope("ph_A"):
            moments = lax.fori_loop(1, NP, scoped("ph_Ai", z2_step), moments)
        stats = z2_stats(moments)
        for r in range(0, FQ, Z2_ROWS):
            z2_operands(NP - 1, (NP - 1) % 2, r, stats)

        mix_pieces = [(r, n) for r in range(0, TB, 16) for n in range(KH // PB)]

        def mix_operands(g, slot, r, n):
            quad = []
            for q in range(4):
                r0 = slot * PB + q % 2 * TB + r
                quad.append(wsp_v[g, r0:r0 + 16, _tile(2 * n + q // 2)])
            quad = [w.astype(F32) for w in quad]
            for k, (_, b_terms, _) in enumerate(STRASSEN):
                (wmix0_v, wmix1_v)[slot][k, n, r:r + 16, :] = _signed_sum(b_terms, quad).astype(BF16)

        def weight_units(g):
            wo_src = wo_u.at[:, _aligned(g * HG * E, HG * E, 32)]

            def split_heads(m, p, r):
                even = raw_u[g, m, p, pl.ds(r, 16, stride=2), :]
                odd = raw_u[g, m, p, pl.ds(r + 1, 16, stride=2), :]
                words = (even & 0xFFFF) | (odd << 16), (even >> 16) | (odd & jnp.uint32(0xFFFF0000))
                for i, w in enumerate(words):
                    big_u[_aligned((m * HP + g * HG) * (D // 2) + (p * D + r) // 2, 16, 8), _tile(i)] = w
                return words

            def store_sums(words, m, p, r, c):
                quad = [pltpu.bitcast(w, BF16).astype(F32) for w in words]
                for n, k in enumerate(SUMMED):
                    rows = _aligned(ROW_SUM + (m * HP + g * HG) * NSUM + (p * NSUM + n * E // 2 + r), 16, 8)
                    big_u[rows, _tile(c)] = pltpu.bitcast(_signed_sum(STRASSEN[k][1], quad).astype(BF16), U32)

            def qkv_unit(m, p, r):
                if r >= DS:
                    split_heads(m, p, r)
                else:
                    store_sums(split_heads(m, p, r) + split_heads(m, p, r + DS // 2), m, p, r % E // 2, r // E)

            def wo_unit(p, c, r):
                words = [wo_src[q % 2 * CS + c, pl.ds((2 * p + q // 2) * E // 2 + r, 16), :] for q in range(4)]
                store_sums(words, 3, p, r, c)

            def wout_unit(n):
                block = jnp.minimum(g * WG + n, NW - 1)
                cols = _aligned(block % DT * LANES, LANES, LANES)
                w = wout_v[_aligned(block // DT * PB, PB, PB), cols].astype(F32)
                woutt_v[block // DT, cols, :] = w.T.astype(BF16)

            units = [functools.partial(qkv_unit, m, p, r) for m in range(3) for p in range(HG)
                     for r in (*range(0, DS // 2, 32), *range(DS, D, 32))]
            units += [functools.partial(wo_unit, p, c, r) for p in range(HG) for c in range(CS)
                      for r in range(0, E // 2, 16)]
            return units, [functools.partial(wout_unit, n) for n in range(WG)]

        def mix_step(second, g, carry):
            nxt = jnp.minimum(g + 1, 2 * NG - 1)
            wait_filled(raw_u.at[g], sem_raw.at[g])
            _wait(cp_wo(g))
            pl.when(g + 1 < 2 * NG)(lambda: wait_filled(wsp_v.at[nxt], sem_sp.at[nxt]))
            for n in range(second * NG, min((second + 1) * NG, 2 * NG - 2)):
                pl.when(g == n)(lambda: _start(cp_group(n + 3) if n + 3 < 2 * NG else cp_win(0)))

            units, extra = weight_units(g)
            if second:
                for n, unit in enumerate(extra):
                    units.insert((2 * n + 1) * len(units) // (2 * len(extra)), unit)
            else:
                units += extra
            chunks = mix_rows[second]
            after = cfg.get("after", (1, 3, 5))
            slots, done = 2 * len(chunks) * len(after), 0
            for t in range(2):
                pair = 2 * (g - second * NG) + t
                bias = [bias_v[pl.ds(2 * pair + i, 1), :] for i in range(2)]
                for c, size in enumerate(chunks):
                    r0 = sum(chunks[:c])

                    def where(q):
                        row = ROW_G + 2 * (g - second * NG) * FH + (t * FH + q // 2 * FQ + r0)
                        return _aligned(row, size, 8), _tile(q % 2)

                    sums = {}
                    for k, (_, _, c_terms) in enumerate(STRASSEN):
                        pairs = range(KH // PB)
                        prod = _dot_nt(
                            jnp.concatenate([z2_v[second * len(pairs) + n, k, r0:r0 + size, :] for n in pairs], axis=1),
                            jnp.concatenate([(wmix0_v, wmix1_v)[t][k, n] for n in pairs], axis=1))
                        for q, sign in c_terms:
                            if q not in sums:
                                sums[q] = pltpu.bitcast(big_u[where(q)], F32) if second else bias[q % 2]
                            _accumulate(sums, q, prod, sign)
                            if all(q != later for _, _, terms in STRASSEN[k + 1:] for later, _ in terms):
                                big_u[where(q)] = pltpu.bitcast(sums[q], U32)
                        if k in after:
                            for unit in units[done * len(units) // slots:(done + 1) * len(units) // slots]:
                                unit()
                            n = done - t * slots // 2
                            wsp_v[jnp.maximum(g, 2 * NG), 0:8, 0:PB] = (
                                jnp.concatenate([prod[0:8]] * 2, axis=1).astype(BF16))
                            for piece in mix_pieces[2 * n * len(mix_pieces) // slots:
                                                    2 * (n + 1) * len(mix_pieces) // slots]:
                                mix_operands(nxt if t else g, 1 - t, *piece)
                            done += 1
            return carry

        _wait(cp_small())
        bias_v[...] = bsp_v[...].astype(F32)
        wait_filled(wsp_v.at[0], sem_sp.at[0])
        for piece in mix_pieces:
            mix_operands(0, 0, *piece)
        with scope("ph_B"):
            for second in range(2):
                lax.fori_loop(second * NG, (second + 1) * NG, scoped("ph_Bi", functools.partial(mix_step, second)), 0)
        _wait(cp_win(0))

        def finish(j, c):
            half_gate = 0.5 * gate_v[_tile(c), :]
            gate = (half_gate + half_gate * jnp.tanh(half_gate)).T
            x = x_v[_aligned(j * TB, TB, TB), _tile(c)].astype(F32)
            xo_v[_aligned(S + j * TB, TB, TB), _tile(c)] = (x + s_v[j % 2, :, _tile(c)] * gate).astype(BF16)

        def scan_tile(j, mem):
            xn_tile = xo_v[_aligned(j * TB, TB, TB), :]

            def side_piece(kind, r0, r1):
                if kind == "out":
                    for c in range(r0, r1):
                        finish(jnp.maximum(j - 1, 0), c)
                elif kind == "z1":
                    g2 = pltpu.bitcast(big_u[_aligned(ROW_G + j // 2 * FH + r0, r1 - r0, 8), :], F32)
                    g = jnp.where(j % 2 == 0, g2[:, _tile(0)], g2[:, _tile(1)])
                    y_v[r0:r1, :] = (z_rows(0, r0, r1, xn_tile) * (0.5 * g)).astype(BF16)
                else:
                    w = jnp.concatenate([woutt_v[n // 2, r0:r1, _tile(n % 2)] for n in range(FT)], axis=1)
                    gate_v[r0:r1, :] = _dot(w, y_v[...])

            row = lax.broadcasted_iota(jnp.int32, (M + SEG, M + SEG), 0)
            col = lax.broadcasted_iota(jnp.int32, (M + SEG, M + SEG), 1)
            visible = (row < M) | (row >= col)
            zero = jnp.minimum(j, 0)

            def put(slot, rows):
                ahead_v[zero + slot, 0:rows.shape[0], :] = rows

            def get(slot, n):
                return [ahead_v[zero + slot, 0:n, :]] if n else []

            for u in range(SPB):
                r0 = SEG + u * (SEG - M) if u else 0
                r1 = SEG + (u + 1) * (SEG - M)
                lo, hi = r0 // 16 * 16, -(-r1 // 16) * 16
                tokens = xo_v[_aligned(j * TB + lo, hi - lo, 16), :].astype(F32)[r0 - lo:r1 - lo]
                h = jnp.concatenate([mem, tokens], axis=0)
                qkv, scores, heads, sums = {}, {}, {}, {}

                def keep(m, hd, rows):
                    early = r0 - u * SEG
                    qkv[m, hd] = jnp.concatenate(
                        [rows[0:M]] + get(3 * hd + m, early) + [rows[M:M + SEG - early]], axis=0)
                    if M + SEG - early < rows.shape[0]:
                        put(3 * hd + m, rows[M + SEG - early:])

                def project_pair(m, hp):
                    out = {}
                    for i in range(2):
                        rest = _dot(h[:, DS:D], w_head(m * H + 2 * hp + i, DS, D))
                        for n in range(2):
                            _accumulate(out, 2 * n + i, rest[n * SEG:(n + 1) * SEG])
                    for k, (_, b_terms, c_terms) in enumerate(STRASSEN):
                        if k in SUMMED:
                            w = jnp.concatenate([w_sum(m, hp, k, c) for c in range(CS)], axis=0)
                        else:
                            q = b_terms[0][0]
                            w = w_head(m * H + 2 * hp + q % 2, q // 2 * (DS // 2), (q // 2 + 1) * (DS // 2))
                        prod = _dot(h_sums[k], w)
                        for q, sign in c_terms:
                            _accumulate(out, q, prod, sign)
                    for i in range(2):
                        keep(m, 2 * hp + i, jnp.concatenate([out[i], out[2 + i]], axis=0))

                def out_rows(hd):
                    rows, late = heads.pop(hd), u * M
                    new = (2 * SEG if u == SPB - 1 else SEG) - M - late
                    lhs = jnp.concatenate([rows[0:M]] + get(3 * H + hd, late) + [rows[M:M + new]], axis=0)
                    if new < SEG:
                        put(3 * H + hd, rows[M + new:])
                    return lhs

                def out_pair(hp):
                    lhs = [out_rows(2 * hp + i) for i in range(2)]
                    quad = [lhs[q % 2][q // 2 * SEG:(q // 2 + 1) * SEG] for q in range(4)]
                    for i in range(2):
                        for c in range(2 * CS, DT):
                            _accumulate(sums, c, _dot(lhs[i], wo_head(2 * hp + i, c)))
                    for k, (a_terms, b_terms, _) in enumerate(STRASSEN):
                        a_sum = _signed_sum(a_terms, quad)
                        for c in range(CS):
                            if k in SUMMED:
                                w = w_sum(3, hp, k, c)
                            else:
                                q = b_terms[0][0]
                                w = wo_head(2 * hp + q // 2, q % 2 * CS + c)
                            _accumulate(sums, (k, c), _dot(a_sum, w))

                if u == 0:
                    quad = [h[q // 2 * SEG:(q // 2 + 1) * SEG, q % 2 * (DS // 2):(q % 2 + 1) * (DS // 2)]
                            for q in range(4)]
                    h_sums = [_signed_sum(a_terms, quad) for a_terms, _, _ in STRASSEN]
                for t in range(H + LAG_OUT):
                    if t < H and u == 0:
                        for m in ((1, 0), (2,))[t % 2]:
                            project_pair(m, t // 2)
                    elif t < H:
                        for m in (1, 0, 2):
                            keep(m, t, _dot(h, w_head(m * H + t)))
                    hd = t - LAG_SCORES
                    if 0 <= hd < H:
                        scores[hd] = _dot_nt(qkv.pop((0, hd)), qkv.pop((1, hd)).astype(BF16))
                    hd = t - LAG_VALUES
                    if 0 <= hd < H:
                        s = jnp.where(visible, scores.pop(hd) * (E ** -0.5 * LOG2E), -1e9 * LOG2E)
                        e = jnp.exp2(s - jnp.max(s, axis=-1, keepdims=True))
                        norm = _reciprocal(jnp.sum(e, axis=-1, keepdims=True))
                        heads[hd] = _dot(e, qkv.pop((2, hd)).astype(BF16)) * norm
                    hd = t - LAG_OUT
                    if 0 <= hd < H and u < SPB - 1:
                        lhs = out_rows(hd)
                        for c in range(DT):
                            _accumulate(sums, c, _dot(lhs, wo_head(hd, c)))
                    elif 0 <= hd < H and hd % 2:
                        out_pair(hd // 2)
                    for piece in side_work.get((u, t), ()):
                        side_piece(*piece)
                if u == SPB - 1:
                    for c in range(CS):
                        out = {}
                        for k, (_, _, c_terms) in enumerate(STRASSEN):
                            for q, sign in c_terms:
                                _accumulate(out, q, sums[k, c], sign)
                        for i in range(2):
                            sums[i * CS + c] = jnp.concatenate([out[i], out[2 + i]], axis=0)
                mem = jnp.concatenate([sums[c][0:M] for c in range(DT)], axis=1)
                for c in range(DT):
                    first = u * (SEG - M)
                    s_v[j % 2, first:first + sums[c].shape[0] - M, _tile(c)] = sums[c][M:]

            @pl.when(j > 0)
            def _():
                pltpu.make_async_copy(xo_v.at[_aligned(S + (j - 1) * TB, TB, TB)],
                                      o_hbm.at[_aligned((j - 1) * TB, TB, TB)], sem_out.at[0]).start()

            return mem

        with scope("ph_main"):
            lax.fori_loop(0, NB, scan_tile, mem_v[...].astype(F32))
        for c in range(DT):
            finish(NB - 1, c)
            cols = pl.ds(c * LANES, LANES)
            pltpu.make_async_copy(xo_v.at[pl.ds(2 * S - TB, TB), cols], o_hbm.at[pl.ds(S - TB, TB), cols],
                                  sem_out.at[0]).start()
        wait_filled(o_hbm, sem_out.at[0])

    scratch = [
        pltpu.VMEM((S, D), BF16),
        pltpu.VMEM((2 * S, D), BF16),
        pltpu.VMEM((2, DT, FH // 2, LANES), U32),
        pltpu.VMEM((2 * NG, 3, HG, D, E), U32),
        pltpu.VMEM((ROWS + cfg.get("pad", 8), 2 * LANES), U32),
        pltpu.VMEM((DT, H * E // 2, LANES), U32),
        pltpu.VMEM((2 * NG + 1, 2 * PB, KH), BF16),
        pltpu.VMEM((7, KH // PB, TB, TB), BF16),
        pltpu.VMEM((7, KH // PB, TB, TB), BF16),
        pltpu.VMEM((5, FH, TB), F32),
        pltpu.VMEM((NP, 7, FQ, TB), BF16),
        pltpu.VMEM((FP, D), BF16),
        pltpu.VMEM((FP // PB, D, PB), BF16),
        pltpu.VMEM((M, D), BF16),
        pltpu.VMEM((NB, TB), BF16),
        pltpu.VMEM((NB, TB), F32),
        pltpu.VMEM((FT * LANES, TB), BF16),
        pltpu.VMEM((D, TB), F32),
        pltpu.VMEM((2, TB, D), F32),
        pltpu.VMEM((4 * H, SEG - M, E), F32),
        pltpu.SemaphoreType.DMA((NP,)),
        pltpu.SemaphoreType.DMA((3,)),
        pltpu.SemaphoreType.DMA((3,)),
        pltpu.SemaphoreType.DMA((2 * NG,)),
        pltpu.SemaphoreType.DMA((2 * NG,)),
        pltpu.SemaphoreType.DMA((2 * NG,)),
        pltpu.SemaphoreType.DMA((1,)),
    ]
    return kernel, scratch, 2 * NG


def build(cfg=None, name="rmt_gmlp"):
    def fn(A_x, A_mem0, A_Wq, A_Wk, A_Wv, A_Wo, A_seg_len, B_x, B_w_in, B_w_sp, B_b_sp, B_w_out):
        del B_x
        B, S, D = A_x.shape
        _, H, E = A_Wq.shape
        M = A_mem0.shape[1]
        assert B == 1 and E == LANES
        kernel, scratch, groups = _make_kernel(S, D, H, M, int(A_seg_len), B_w_out.shape[0], cfg or {})
        hbm = pl.BlockSpec(memory_space=pltpu.HBM)
        out = pl.pallas_call(
            kernel,
            out_shape=jax.ShapeDtypeStruct((S, D), A_x.dtype),
            in_specs=[hbm] * 10,
            out_specs=hbm,
            scratch_shapes=scratch,
            compiler_params=pltpu.CompilerParams(vmem_limit_bytes=120 * 1024 * 1024),
            name=name,
        )(A_x.reshape(S, D), A_mem0.reshape(M, D),
          *(w.reshape(D, groups, H // groups, E) for w in (A_Wq, A_Wk, A_Wv)), A_Wo.reshape(H * E, D),
          B_w_in.T, B_w_sp, B_b_sp.reshape(S // LANES, LANES), B_w_out)
        return out.reshape(B, S, D)

    return fn


pallas_recurrent_scan__memory_aug_recurrent_mem_tr__mixer_gmlp__prompt_kernel = jax.jit(
    build(), static_argnames=("A_seg_len",))
```

```python
import functools
import math

import jax
import jax.numpy as jnp
from jax import lax
import jax.experimental.pallas as pl
import jax.experimental.pallas.tpu as pltpu

F32, BF16, U32 = jnp.float32, jnp.bfloat16, jnp.uint32
LANES = 128
EPS = 1e-5
LOG2E = math.log2(math.e)

STRASSEN = (
    (((0, 1), (3, 1)), ((0, 1), (3, 1)), ((0, 1), (3, 1))),
    (((3, 1),), ((2, 1), (0, -1)), ((0, 1), (2, 1))),
    (((0, 1), (1, 1)), ((3, 1),), ((0, -1), (1, 1))),
    (((1, 1), (3, -1)), ((2, 1), (3, 1)), ((0, 1),)),
    (((0, 1),), ((1, 1), (3, -1)), ((1, 1), (3, 1))),
    (((2, 1), (3, 1)), ((0, 1),), ((2, 1), (3, -1))),
    (((2, 1), (0, -1)), ((0, 1), (1, 1)), ((3, 1),)),
)
SUMMED = tuple(k for k, (_, b_terms, _) in enumerate(STRASSEN) if len(b_terms) > 1)

LAG_SCORES, LAG_VALUES, LAG_OUT = 1, 3, 4


def _lay_out(steps):
    end, plan = {}, {}
    for u, pieces in enumerate(steps):
        for slot, kind, size in pieces:
            start = end.get(kind, 0)
            end[kind] = start + size
            plan.setdefault((u, slot), []).append((kind, start, start + size))
    return plan, end


SIDE_WORK = (
    ((8, "out", 1), (16, "out", 1), (28, "out", 1),
     (31, "z1", 96), (32, "z1", 80), (33, "z1", 80), (34, "z1", 64), (35, "z1", 112)),
    ((6, "out", 1), (31, "z1", 96), (32, "z1", 64), (33, "z1", 112), (34, "z1", 80), (35, "z1", 80)),
    ((7, "out", 1), (31, "w_out", 96), (32, "w_out", 64), (33, "w_out", 48), (34, "w_out", 48), (35, "w_out", 80)),
    ((32, "w_out", 96), (33, "w_out", 48), (34, "w_out", 112), (35, "w_out", 48)),
)
Z2_ROWS = 144
MIX_ROWS = ((80, 80, 80, 96, 96), (96, 96, 80, 80, 80))


def _dot(a, b):
    return jnp.dot(a, b, preferred_element_type=F32)


def _dot_nt(a, b):
    return lax.dot_general(a, b, (((1,), (1,)), ((), ())), preferred_element_type=F32)


def _twice_gelu(x):
    c = math.sqrt(2.0 / math.pi)
    return x + x * jnp.tanh(x * (x * x * (0.044715 * c) + c))


def _reciprocal(x):
    r = pltpu.reciprocal(x, approx=True)
    return r * (2.0 - x * r)


def _tree_sum(xs):
    xs = list(xs)
    while len(xs) > 1:
        xs = [xs[i] + xs[i + 1] if i + 1 < len(xs) else xs[i] for i in range(0, len(xs), 2)]
    return xs[0]


def _signed_sum(terms, blocks):
    (first, _), *rest = terms
    total = blocks[first]
    for q, sign in rest:
        total = total + blocks[q] if sign > 0 else total - blocks[q]
    return total


def _accumulate(sums, key, value, sign=1):
    if key in sums:
        sums[key] = sums[key] + value if sign > 0 else sums[key] - value
    else:
        sums[key] = value if sign > 0 else -value


def _aligned(start, size, unit):
    return pl.ds(start if isinstance(start, int) else pl.multiple_of(start, unit), size)


def _tile(i):
    return slice(i * LANES, (i + 1) * LANES)


def _start(copies):
    for c in copies:
        c.start()


def _wait(copies):
    for c in copies:
        c.wait()


def _make_kernel(S, D, H, M, SEG, FH):
    E = TB = LANES
    PB = 2 * TB
    NB, NP = S // TB, S // PB
    SPB = TB // SEG
    DT = D // LANES
    DS = D // PB * PB
    CS = DS // PB
    FQ = FH // 2
    FT = -(-FH // LANES)
    FP = -(-FH // PB) * PB
    KH = S // 2
    NG = NP // 2
    HP = H // 2
    HG = HP // (2 * NG)
    NW = FP // PB * DT
    WG = -(-NW // (2 * NG))
    NSUM = len(SUMMED) * E // 2
    ROW_G = 3 * HP * D // 2
    ROW_SUM = ROW_G + NP * FH
    ROWS = ROW_SUM + 4 * HP * NSUM
    side_work, side_total = _lay_out(SIDE_WORK)
    assert side_total == {"out": DT, "z1": FH, "w_out": D} and all(sum(r) == FQ for r in MIX_ROWS)
    assert CS == 2 and SPB == 4 and SEG == SPB * M and FQ % Z2_ROWS == 0 and HP == 2 * NG * HG

    def kernel(x_hbm, mem_hbm, wq_hbm, wk_hbm, wv_hbm, wo_hbm, win_hbm, wsp_hbm, bsp_hbm, wout_hbm,
               o_hbm,
               x_v, xo_v, win_u, raw_u, big_u, wo_u, wsp_v, wmix0_v, wmix1_v, zraw_v, z2_v,
               wout_v, woutt_v, mem_v, bsp_v, bias_v, y_v, gate_v, s_v, ahead_v,
               sem_x, sem_win, sem_small, sem_raw, sem_sp, sem_wo, sem_out):

        def w_head(n, d0=0, d1=D):
            return pltpu.bitcast(big_u[(n // 2 * D + d0) // 2:(n // 2 * D + d1) // 2, _tile(n % 2)], BF16)

        def w_sum(m, hp, k, c):
            row = ROW_SUM + (m * HP + hp) * NSUM + SUMMED.index(k) * E // 2
            return pltpu.bitcast(big_u[row:row + E // 2, _tile(c)], BF16)

        def wo_head(hd, c):
            return pltpu.bitcast(wo_u[c, hd * E // 2:(hd + 1) * E // 2, :], BF16)

        def cp_x(p):
            rows = _aligned(p * PB, PB, PB)
            return pltpu.make_async_copy(x_hbm.at[rows], x_v.at[rows], sem_x.at[p])

        def cp_win(half, part=0, parts=1):
            n = FH // 2 // parts
            return [pltpu.make_async_copy(
                win_hbm.bitcast(U32).at[pl.ds(half * FH // 2 + part * n, n), pl.ds(c * LANES, LANES)],
                win_u.at[half, c, pl.ds(part * n, n)], sem_win.at[half + part]) for c in range(DT)]

        def cp_small():
            return [pltpu.make_async_copy(mem_hbm, mem_v, sem_small.at[0]),
                    pltpu.make_async_copy(bsp_hbm, bsp_v, sem_small.at[1]),
                    pltpu.make_async_copy(wout_hbm, wout_v.at[pl.ds(0, FH)], sem_small.at[2])]

        def cp_wo(g):
            rows = _aligned(g * HG * E, HG * E, HG * E)
            return [pltpu.make_async_copy(wo_hbm.bitcast(U32).at[rows, pl.ds(c * LANES, LANES)],
                                          wo_u.at[c, rows], sem_wo.at[g]) for c in range(DT)]

        def cp_group(g):
            copies = [pltpu.make_async_copy(
                wsp_hbm.at[pl.ds(n % NG * 2 * PB, 2 * PB), pl.ds(n // NG * KH, KH)], wsp_v.at[n], sem_sp.at[n])
                for n in range(g + 1 if g else 0, min(g + 2, 2 * NG))]
            for m, w_hbm in enumerate((wq_hbm, wk_hbm, wv_hbm)):
                copies += [pltpu.make_async_copy(w_hbm.bitcast(U32).at[:, g, p, :], raw_u.at[g, m, p], sem_raw.at[g])
                           for p in range(HG)]
            return copies + cp_wo(g)

        def wait_filled(buf, sem):
            pltpu.make_async_copy(buf, buf, sem).wait()

        def layernorm_rows(r0, n):
            rows = _aligned(r0, n, n)
            x = x_v[rows, :].astype(F32)
            d = x - jnp.sum(x, axis=-1, keepdims=True) * (1.0 / D)
            xn = d * lax.rsqrt(jnp.sum(d * d, axis=-1, keepdims=True) * (1.0 / D) + EPS)
            xo_v[rows, :] = xn.astype(BF16)
            return xn

        def z_rows(half, r0, r1, xn):
            w = jnp.concatenate([pltpu.bitcast(win_u[half, c, r0 // 2:r1 // 2, :], BF16) for c in range(DT)], axis=1)
            return _twice_gelu(_dot_nt(w, xn))

        def z2_stats(moments):
            stats = []
            for means, m2 in moments:
                mu = jnp.sum(_tree_sum(means), axis=0, keepdims=True) * (1.0 / (8 * len(means)))
                m2 = m2 + (Z2_ROWS // 8) * _tree_sum((m - mu) * (m - mu) for m in means)
                rs = lax.rsqrt(jnp.sum(m2, axis=0, keepdims=True) * (1.0 / FH) + 4 * EPS)
                stats.append((jnp.broadcast_to(mu, (8, TB)), jnp.broadcast_to(rs, (8, TB))))
            return stats

        def z2_operands(p, slot, r, stats):
            quad = []
            for q in range(4):
                mu, rs = stats[q % 2]
                r0 = r + q // 2 * FQ
                z = zraw_v[2 * slot + q % 2, r0:r0 + Z2_ROWS, :].reshape(Z2_ROWS // 8, 8, TB)
                quad.append(((z - mu) * rs).reshape(Z2_ROWS, TB))
            for k, (a_terms, _, _) in enumerate(STRASSEN):
                z2_v[p, k, r:r + Z2_ROWS, :] = _signed_sum(a_terms, quad).astype(BF16)

        def z2_pair(p, prev_moments):
            opening = prev_moments is None
            nxt = p + 1 if opening else jnp.minimum(p + 1, NP - 1)
            prev_stats = None if opening else z2_stats(prev_moments)
            xn = [xo_v[_aligned(p * PB + t * TB, TB, TB), :] for t in range(2)]
            order = [(t, r) for t in range(2) for r in range(0, FH, Z2_ROWS)]
            if opening:
                order.sort(key=lambda tr: tr[1])
            steps, n_norm, n_ops = len(order), PB // 64, FQ // Z2_ROWS
            means, m2 = ([], []), {}
            for n, (t, r) in enumerate(order):
                if opening and n == steps // 2:
                    _wait(cp_win(1, 1, 2) + [cp_x(1)])
                    _start([cp_x(i) for i in range(2, NP)] + cp_small())
                z = z_rows(1, r, r + Z2_ROWS, xn[t])
                zraw_v[2 * (p % 2) + t, r:r + Z2_ROWS, :] = z
                parts = [z[i:i + 8] for i in range(0, Z2_ROWS, 8)]
                mean = _tree_sum(parts) * (1.0 / len(parts))
                _accumulate(m2, t, _tree_sum((v - mean) * (v - mean) for v in parts))
                means[t].append(mean)
                if opening:
                    late = max(0, n + 1 - steps // 2)
                    for i in range(max(0, late - 1) * n_norm // (steps // 2), late * n_norm // (steps // 2)):
                        layernorm_rows(nxt * PB + i * 64, 64)
                    continue
                for i in range(n * n_norm // steps, (n + 1) * n_norm // steps):
                    rows = layernorm_rows(nxt * PB + i * 64, 64)
                    zraw_v[jnp.maximum(p % 2, 4), 0:64, :] = rows[:, D - LANES:D]
                for i in range(n * n_ops // steps, (n + 1) * n_ops // steps):
                    z2_operands(p - 1, 1 - p % 2, i * Z2_ROWS, prev_stats)
            return tuple((tuple(means[t]), m2[t]) for t in range(2))

        def z2_step(p, moments):
            pl.when(p + 1 < NP)(lambda: cp_x(jnp.minimum(p + 1, NP - 1)).wait())
            pl.when(p == NP // 2 - 1)(lambda: _start(cp_group(1)))
            return z2_pair(p, moments)

        _start([cp_x(0)] + cp_win(1, 0, 2))
        wout_v[FH:FP, :] = jnp.zeros((FP - FH, D), BF16)
        y_v[FH:FT * LANES, :] = jnp.zeros((FT * LANES - FH, TB), BF16)
        s_v[...] = jnp.zeros(s_v.shape, F32)
        gate_v[...] = jnp.zeros(gate_v.shape, F32)
        cp_x(0).wait()
        _start(cp_win(1, 1, 2) + [cp_x(1)])
        _wait(cp_win(1, 0, 2))
        for r in range(0, PB, 32):
            layernorm_rows(r, 32)
        moments = z2_pair(0, None)
        _start(cp_group(0))
        moments = lax.fori_loop(1, NP, z2_step, moments)
        _start(cp_group(2))
        stats = z2_stats(moments)
        for r in range(0, FQ, Z2_ROWS):
            z2_operands(NP - 1, (NP - 1) % 2, r, stats)

        mix_pieces = [(r, n) for r in range(0, TB, 16) for n in range(KH // PB)]

        def mix_operands(g, slot, r, n):
            quad = []
            for q in range(4):
                r0 = slot * PB + q % 2 * TB + r
                quad.append(wsp_v[g, r0:r0 + 16, _tile(2 * n + q // 2)])
            quad = [w.astype(F32) for w in quad]
            for k, (_, b_terms, _) in enumerate(STRASSEN):
                (wmix0_v, wmix1_v)[slot][k, n, r:r + 16, :] = _signed_sum(b_terms, quad).astype(BF16)

        def weight_units(g):
            wo_src = wo_u.at[:, _aligned(g * HG * E, HG * E, 32)]

            def split_heads(m, p, r):
                even = raw_u[g, m, p, pl.ds(r, 16, stride=2), :]
                odd = raw_u[g, m, p, pl.ds(r + 1, 16, stride=2), :]
                words = (even & 0xFFFF) | (odd << 16), (even >> 16) | (odd & jnp.uint32(0xFFFF0000))
                for i, w in enumerate(words):
                    big_u[_aligned((m * HP + g * HG) * (D // 2) + (p * D + r) // 2, 16, 8), _tile(i)] = w
                return words

            def store_sums(words, m, p, r, c):
                quad = [pltpu.bitcast(w, BF16).astype(F32) for w in words]
                for n, k in enumerate(SUMMED):
                    rows = _aligned(ROW_SUM + (m * HP + g * HG) * NSUM + (p * NSUM + n * E // 2 + r), 16, 8)
                    big_u[rows, _tile(c)] = pltpu.bitcast(_signed_sum(STRASSEN[k][1], quad).astype(BF16), U32)

            def qkv_unit(m, p, r):
                if r >= DS:
                    split_heads(m, p, r)
                else:
                    store_sums(split_heads(m, p, r) + split_heads(m, p, r + DS // 2), m, p, r % E // 2, r // E)

            def wo_unit(p, c, r):
                words = [wo_src[q % 2 * CS + c, pl.ds((2 * p + q // 2) * E // 2 + r, 16), :] for q in range(4)]
                store_sums(words, 3, p, r, c)

            def wout_unit(n):
                block = jnp.minimum(g * WG + n, NW - 1)
                cols = _aligned(block % DT * LANES, LANES, LANES)
                w = wout_v[_aligned(block // DT * PB, PB, PB), cols].astype(F32)
                woutt_v[block // DT, cols, :] = w.T.astype(BF16)

            units = [functools.partial(qkv_unit, m, p, r) for m in range(3) for p in range(HG)
                     for r in (*range(0, DS // 2, 32), *range(DS, D, 32))]
            units += [functools.partial(wo_unit, p, c, r) for p in range(HG) for c in range(CS)
                      for r in range(0, E // 2, 16)]
            return units, [functools.partial(wout_unit, n) for n in range(WG)]

        def mix_step(second, g, carry):
            nxt = jnp.minimum(g + 1, 2 * NG - 1)
            wait_filled(raw_u.at[g], sem_raw.at[g])
            _wait(cp_wo(g))
            pl.when(g + 1 < 2 * NG)(lambda: wait_filled(wsp_v.at[nxt], sem_sp.at[nxt]))
            for n in range(second * NG, min((second + 1) * NG, 2 * NG - 2)):
                pl.when(g == n)(lambda: _start(cp_group(n + 3) if n + 3 < 2 * NG else cp_win(0)))

            units, extra = weight_units(g)
            if second:
                for n, unit in enumerate(extra):
                    units.insert((2 * n + 1) * len(units) // (2 * len(extra)), unit)
            else:
                units += extra
            chunks = MIX_ROWS[second]
            after = (1, 3, 5)
            slots, done = 2 * len(chunks) * len(after), 0
            for t in range(2):
                pair = 2 * (g - second * NG) + t
                bias = [bias_v[pl.ds(2 * pair + i, 1), :] for i in range(2)]
                for c, size in enumerate(chunks):
                    r0 = sum(chunks[:c])

                    def where(q):
                        row = ROW_G + 2 * (g - second * NG) * FH + (t * FH + q // 2 * FQ + r0)
                        return _aligned(row, size, 8), _tile(q % 2)

                    sums = {}
                    for k, (_, _, c_terms) in enumerate(STRASSEN):
                        pairs = range(KH // PB)
                        prod = _dot_nt(
                            jnp.concatenate([z2_v[second * len(pairs) + n, k, r0:r0 + size, :] for n in pairs], axis=1),
                            jnp.concatenate([(wmix0_v, wmix1_v)[t][k, n] for n in pairs], axis=1))
                        for q, sign in c_terms:
                            if q not in sums:
                                sums[q] = pltpu.bitcast(big_u[where(q)], F32) if second else bias[q % 2]
                            _accumulate(sums, q, prod, sign)
                            if all(q != later for _, _, terms in STRASSEN[k + 1:] for later, _ in terms):
                                big_u[where(q)] = pltpu.bitcast(sums[q], U32)
                        if k in after:
                            for unit in units[done * len(units) // slots:(done + 1) * len(units) // slots]:
                                unit()
                            n = done - t * slots // 2
                            wsp_v[jnp.maximum(g, 2 * NG), 0:8, 0:PB] = (
                                jnp.concatenate([prod[0:8]] * 2, axis=1).astype(BF16))
                            for piece in mix_pieces[2 * n * len(mix_pieces) // slots:
                                                    2 * (n + 1) * len(mix_pieces) // slots]:
                                mix_operands(nxt if t else g, 1 - t, *piece)
                            done += 1
            return carry

        _wait(cp_small())
        bias_v[...] = bsp_v[...].astype(F32)
        wait_filled(wsp_v.at[0], sem_sp.at[0])
        for piece in mix_pieces:
            mix_operands(0, 0, *piece)
        for second in range(2):
            lax.fori_loop(second * NG, (second + 1) * NG, functools.partial(mix_step, second), 0)
        _wait(cp_win(0))

        def finish(j, c):
            half_gate = 0.5 * gate_v[_tile(c), :]
            gate = (half_gate + half_gate * jnp.tanh(half_gate)).T
            x = x_v[_aligned(j * TB, TB, TB), _tile(c)].astype(F32)
            xo_v[_aligned(S + j * TB, TB, TB), _tile(c)] = (x + s_v[j % 2, :, _tile(c)] * gate).astype(BF16)

        def scan_tile(j, mem):
            xn_tile = xo_v[_aligned(j * TB, TB, TB), :]

            def side_piece(kind, r0, r1):
                if kind == "out":
                    for c in range(r0, r1):
                        finish(jnp.maximum(j - 1, 0), c)
                elif kind == "z1":
                    g2 = pltpu.bitcast(big_u[_aligned(ROW_G + j // 2 * FH + r0, r1 - r0, 8), :], F32)
                    g = jnp.where(j % 2 == 0, g2[:, _tile(0)], g2[:, _tile(1)])
                    y_v[r0:r1, :] = (z_rows(0, r0, r1, xn_tile) * (0.5 * g)).astype(BF16)
                else:
                    w = jnp.concatenate([woutt_v[n // 2, r0:r1, _tile(n % 2)] for n in range(FT)], axis=1)
                    gate_v[r0:r1, :] = _dot(w, y_v[...])

            row = lax.broadcasted_iota(jnp.int32, (M + SEG, M + SEG), 0)
            col = lax.broadcasted_iota(jnp.int32, (M + SEG, M + SEG), 1)
            visible = (row < M) | (row >= col)
            zero = jnp.minimum(j, 0)

            def put(slot, rows):
                ahead_v[zero + slot, 0:rows.shape[0], :] = rows

            def get(slot, n):
                return [ahead_v[zero + slot, 0:n, :]] if n else []

            for u in range(SPB):
                r0 = SEG + u * (SEG - M) if u else 0
                r1 = SEG + (u + 1) * (SEG - M)
                lo, hi = r0 // 16 * 16, -(-r1 // 16) * 16
                tokens = xo_v[_aligned(j * TB + lo, hi - lo, 16), :].astype(F32)[r0 - lo:r1 - lo]
                h = jnp.concatenate([mem, tokens], axis=0)
                h_narrow = h.astype(BF16)
                qkv, scores, heads, sums = {}, {}, {}, {}

                def keep(m, hd, rows):
                    early = r0 - u * SEG
                    qkv[m, hd] = jnp.concatenate(
                        [rows[0:M]] + get(3 * hd + m, early) + [rows[M:M + SEG - early]], axis=0)
                    if M + SEG - early < rows.shape[0]:
                        put(3 * hd + m, rows[M + SEG - early:])

                def project_pair(m, hp):
                    out = {}
                    for i in range(2):
                        rest = _dot(h_narrow[:, DS:D], w_head(m * H + 2 * hp + i, DS, D))
                        for n in range(2):
                            _accumulate(out, 2 * n + i, rest[n * SEG:(n + 1) * SEG])
                    for k, (_, b_terms, c_terms) in enumerate(STRASSEN):
                        if k in SUMMED:
                            w = jnp.concatenate([w_sum(m, hp, k, c) for c in range(CS)], axis=0)
                        else:
                            q = b_terms[0][0]
                            w = w_head(m * H + 2 * hp + q % 2, q // 2 * (DS // 2), (q // 2 + 1) * (DS // 2))
                        prod = _dot(h_sums[k], w)
                        for q, sign in c_terms:
                            _accumulate(out, q, prod, sign)
                    for i in range(2):
                        keep(m, 2 * hp + i, jnp.concatenate([out[i], out[2 + i]], axis=0))

                def out_rows(hd):
                    rows, late = heads.pop(hd), u * M
                    new = (2 * SEG if u == SPB - 1 else SEG) - M - late
                    lhs = jnp.concatenate([rows[0:M]] + get(3 * H + hd, late) + [rows[M:M + new]], axis=0)
                    if new < SEG:
                        put(3 * H + hd, rows[M + new:])
                    return lhs

                def out_pair(hp):
                    lhs = [out_rows(2 * hp + i) for i in range(2)]
                    quad = [lhs[q % 2][q // 2 * SEG:(q // 2 + 1) * SEG] for q in range(4)]
                    for i in range(2):
                        for c in range(2 * CS, DT):
                            _accumulate(sums, c, _dot(lhs[i].astype(BF16), wo_head(2 * hp + i, c)))
                    for k, (a_terms, b_terms, _) in enumerate(STRASSEN):
                        a_sum = _signed_sum(a_terms, quad).astype(BF16)
                        for c in range(CS):
                            if k in SUMMED:
                                w = w_sum(3, hp, k, c)
                            else:
                                q = b_terms[0][0]
                                w = wo_head(2 * hp + q // 2, q % 2 * CS + c)
                            _accumulate(sums, (k, c), _dot(a_sum, w))

                if u == 0:
                    quad = [h[q // 2 * SEG:(q // 2 + 1) * SEG, q % 2 * (DS // 2):(q % 2 + 1) * (DS // 2)]
                            for q in range(4)]
                    h_sums = [_signed_sum(a_terms, quad).astype(BF16) for a_terms, _, _ in STRASSEN]
                for t in range(H + LAG_OUT):
                    if t < H and u == 0:
                        for m in ((1, 0), (2,))[t % 2]:
                            project_pair(m, t // 2)
                    elif t < H:
                        for m in (1, 0, 2):
                            keep(m, t, _dot(h_narrow, w_head(m * H + t)))
                    hd = t - LAG_SCORES
                    if 0 <= hd < H:
                        scores[hd] = _dot_nt(qkv.pop((0, hd)), qkv.pop((1, hd)).astype(BF16))
                    hd = t - LAG_VALUES
                    if 0 <= hd < H:
                        s = jnp.where(visible, scores.pop(hd) * (E ** -0.5 * LOG2E), -1e9 * LOG2E)
                        e = jnp.exp2(s - jnp.max(s, axis=-1, keepdims=True))
                        norm = _reciprocal(jnp.sum(e, axis=-1, keepdims=True))
                        heads[hd] = _dot(e, qkv.pop((2, hd)).astype(BF16)) * norm
                    hd = t - LAG_OUT
                    if 0 <= hd < H and u < SPB - 1:
                        lhs = out_rows(hd).astype(BF16)
                        for c in range(DT):
                            _accumulate(sums, c, _dot(lhs, wo_head(hd, c)))
                    elif 0 <= hd < H and hd % 2:
                        out_pair(hd // 2)
                    for piece in side_work.get((u, t), ()):
                        side_piece(*piece)
                if u == SPB - 1:
                    for c in range(CS):
                        out = {}
                        for k, (_, _, c_terms) in enumerate(STRASSEN):
                            for q, sign in c_terms:
                                _accumulate(out, q, sums[k, c], sign)
                        for i in range(2):
                            sums[i * CS + c] = jnp.concatenate([out[i], out[2 + i]], axis=0)
                mem = jnp.concatenate([sums[c][0:M] for c in range(DT)], axis=1)
                for c in range(DT):
                    first = u * (SEG - M)
                    s_v[j % 2, first:first + sums[c].shape[0] - M, _tile(c)] = sums[c][M:]

            @pl.when(j > 0)
            def _():
                pltpu.make_async_copy(xo_v.at[_aligned(S + (j - 1) * TB, TB, TB)],
                                      o_hbm.at[_aligned((j - 1) * TB, TB, TB)], sem_out.at[0]).start()

            return mem

        lax.fori_loop(0, NB, scan_tile, mem_v[...].astype(F32))
        for c in range(DT):
            finish(NB - 1, c)
            cols = pl.ds(c * LANES, LANES)
            pltpu.make_async_copy(xo_v.at[pl.ds(2 * S - TB, TB), cols], o_hbm.at[pl.ds(S - TB, TB), cols],
                                  sem_out.at[0]).start()
        wait_filled(o_hbm, sem_out.at[0])

    scratch = [
        pltpu.VMEM((S, D), BF16),
        pltpu.VMEM((2 * S, D), BF16),
        pltpu.VMEM((2, DT, FH // 2, LANES), U32),
        pltpu.VMEM((2 * NG, 3, HG, D, E), U32),
        pltpu.VMEM((ROWS + 8, 2 * LANES), U32),
        pltpu.VMEM((DT, H * E // 2, LANES), U32),
        pltpu.VMEM((2 * NG + 1, 2 * PB, KH), BF16),
        pltpu.VMEM((7, KH // PB, TB, TB), BF16),
        pltpu.VMEM((7, KH // PB, TB, TB), BF16),
        pltpu.VMEM((5, FH, TB), F32),
        pltpu.VMEM((NP, 7, FQ, TB), BF16),
        pltpu.VMEM((FP, D), BF16),
        pltpu.VMEM((FP // PB, D, PB), BF16),
        pltpu.VMEM((M, D), BF16),
        pltpu.VMEM((NB, TB), BF16),
        pltpu.VMEM((NB, TB), F32),
        pltpu.VMEM((FT * LANES, TB), BF16),
        pltpu.VMEM((D, TB), F32),
        pltpu.VMEM((2, TB, D), F32),
        pltpu.VMEM((4 * H, SEG - M, E), F32),
        pltpu.SemaphoreType.DMA((NP,)),
        pltpu.SemaphoreType.DMA((3,)),
        pltpu.SemaphoreType.DMA((3,)),
        pltpu.SemaphoreType.DMA((2 * NG,)),
        pltpu.SemaphoreType.DMA((2 * NG,)),
        pltpu.SemaphoreType.DMA((2 * NG,)),
        pltpu.SemaphoreType.DMA((1,)),
    ]
    return kernel, scratch, 2 * NG


@functools.partial(jax.jit, static_argnames=("A_seg_len",))
def pallas_recurrent_scan__memory_aug_recurrent_mem_tr__mixer_gmlp__prompt_kernel(
        A_x, A_mem0, A_Wq, A_Wk, A_Wv, A_Wo, A_seg_len, B_x, B_w_in, B_w_sp, B_b_sp, B_w_out):
    del B_x
    B, S, D = A_x.shape
    _, H, E = A_Wq.shape
    M = A_mem0.shape[1]
    assert B == 1 and E == LANES
    kernel, scratch, groups = _make_kernel(S, D, H, M, int(A_seg_len), B_w_out.shape[0])
    hbm = pl.BlockSpec(memory_space=pltpu.HBM)
    out = pl.pallas_call(
        kernel,
        out_shape=jax.ShapeDtypeStruct((S, D), A_x.dtype),
        in_specs=[hbm] * 10,
        out_specs=hbm,
        scratch_shapes=scratch,
        compiler_params=pltpu.CompilerParams(vmem_limit_bytes=120 * 1024 * 1024),
        name="rmt_gmlp",
    )(A_x.reshape(S, D), A_mem0.reshape(M, D),
      *(w.reshape(D, groups, H // groups, E) for w in (A_Wq, A_Wk, A_Wv)), A_Wo.reshape(H * E, D),
      B_w_in.T, B_w_sp, B_b_sp.reshape(S // LANES, LANES), B_w_out)
    return out.reshape(B, S, D)
```
